```python
import jax
import jax.numpy as jnp

def _softmax(x, axis=-1):
    return jax.nn.softmax(x, axis=axis)

def _gelu(x):
    return jax.nn.gelu(x, approximate=True)

def _silu(x):
    return jax.nn.silu(x)

def _sigmoid(x):
    return jax.nn.sigmoid(x)

def _layernorm(x, axis=-1, eps=1e-05):
    m = jnp.mean(x, axis=axis, keepdims=True)
    v = jnp.var(x, axis=axis, keepdims=True)
    return (x - m) / jnp.sqrt(v + eps)

def _scatter_add(tgt, idx, src, axis=0):
    return tgt.at[idx].add(src)

def _segment_sum(src, seg, n):
    return jax.ops.segment_sum(src, seg, n)

class _Rng:

    def __init__(self, key):
        self._k = key

    def _next(self):
        self._k, sub = jax.random.split(self._k)
        return sub

    def normal(self, shape):
        return jax.random.normal(self._next(), shape, dtype=jnp.bfloat16)

    def randint(self, lo, hi, shape):
        return jax.random.randint(self._next(), shape, lo, hi, dtype=jnp.int32)

    def uniform(self, shape, lo=0.0, hi=1.0):
        return jax.random.uniform(self._next(), shape, jnp.bfloat16, lo, hi)

    def permutation(self, n):
        return jax.random.permutation(self._next(), n)
kernel_name = 'recurrent_scan__ssm_conv_h3__mixer_gmlp__prompt'

def setup_inputs():
    _rng = _Rng(jax.random.key(int.from_bytes(__import__("os").urandom(4), "little")))
    _w = lambda a: (lambda t: t.astype(jnp.bfloat16) if jnp.issubdtype(t.dtype, jnp.floating) else t)(jnp.asarray(a))

    def _A_setup():
        B, S, D = (1, 2048, 640)
        ks = 4
        return {'q': _w((lambda *s: _rng.normal(s) * 0.05)(B, S, D)), 'k': _w((lambda *s: _rng.normal(s) * 0.05)(B, S, D)), 'v': _w((lambda *s: _rng.normal(s) * 0.05)(B, S, D)), 'shift_k': _w((lambda *s: _rng.normal(s) * 0.05)(D, ks) * 0.5), 'ssm_k': _w((lambda *s: _rng.normal(s) * 0.05)(D, S) * (1.0 / S ** 0.5)), 'ssm_D': _w((lambda *s: _rng.normal(s) * 0.05)(D))}
    _A_in = _A_setup()

    def _B_setup():
        B, S, D, F = (1, 2048, 640, 1536)
        Fh = F // 2
        return {'x': _w((lambda *s: _rng.normal(s) * 0.05)(B, S, D)), 'w_in': _w((lambda *s: _rng.normal(s) * 0.05)(D, 2 * Fh)), 'w_sp': _w(0.01 * (lambda *s: _rng.normal(s) * 0.05)(S, S)), 'b_sp': _w(1.0 + 0.01 * (lambda *s: _rng.normal(s) * 0.05)(S)), 'w_out': _w((lambda *s: _rng.normal(s) * 0.05)(Fh, D))}
    _B_in = _B_setup()
    return {'A_q': _A_in['q'], 'A_k': _A_in['k'], 'A_v': _A_in['v'], 'A_shift_k': _A_in['shift_k'], 'A_ssm_k': _A_in['ssm_k'], 'A_ssm_D': _A_in['ssm_D'], 'B_x': _B_in['x'], 'B_w_in': _B_in['w_in'], 'B_w_sp': _B_in['w_sp'], 'B_b_sp': _B_in['b_sp'], 'B_w_out': _B_in['w_out']}

def reference(A_q, A_k, A_v, A_shift_k, A_ssm_k, A_ssm_D, B_x, B_w_in, B_w_sp, B_b_sp, B_w_out):

    def _A_ref(q, k, v, shift_k, ssm_k, ssm_D):
        B, S, D = q.shape
        ks = shift_k.shape[-1]
        k_pad = jnp.pad(k, ((0, 0), (ks - 1, 0), (0, 0)))
        k_shift = jnp.zeros_like(k)
        for t in range(ks):
            k_shift = k_shift + k_pad[:, t:t + S, :] * shift_k[:, ks - 1 - t][None, None, :]
        kv = k_shift * v
        L = 2 * S
        kv_pad = jnp.pad(kv, ((0, 0), (0, S), (0, 0)))
        kf_pad = jnp.pad(ssm_k, ((0, 0), (0, S)))
        kv_f = (lambda x, axes=(-2, -1): jnp.fft.rfft2(x.astype(jnp.float32), axes=axes))(kv_pad[:, None, :, :], axes=(1, 2))
        kf_f = (lambda x, axes=(-2, -1): jnp.fft.rfft2(x.astype(jnp.float32), axes=axes))(kf_pad[:, None, :], axes=(1, 2))
        kf_f = (lambda x, *d: x.transpose(*d))(kf_f, 1, 2, 0)
        y_f = kv_f * kf_f[None, :, :, :]
        y = (lambda x, s, axes=(-2, -1): jnp.fft.irfft2(x, s=s, axes=axes).astype(jnp.bfloat16))(y_f, (1, L), axes=(1, 2))[:, 0, :S, :]
        y = y + kv * ssm_D[None, None, :]
        return q * y

    def _B_ref(x, w_in, w_sp, b_sp, w_out):
        B, S, D = x.shape
        F = w_in.shape[-1]
        Fh = F // 2
        z = _gelu(jnp.einsum('bsd,df->bsf', x, w_in))
        z1 = z[..., :Fh].copy()
        z2 = _layernorm(z[..., Fh:], axis=-1)
        g = jnp.einsum('ts,bsf->btf', w_sp, z2) + b_sp[None, :, None]
        return jnp.einsum('bsf,fd->bsd', z1 * g, w_out)
    x = A_q
    xn = _layernorm(x, axis=-1)
    s = _A_ref(xn, A_k, A_v, A_shift_k, A_ssm_k, A_ssm_D)
    g = _silu(_B_ref(xn, B_w_in, B_w_sp, B_b_sp, B_w_out))
    return x + s * g
```

```python
import numpy as np
import jax
import jax.numpy as jnp
import jax.experimental.pallas as pl
import jax.experimental.pallas.tpu as pltpu

S, D, F, FH = 2048, 640, 1536, 768
N1, N2 = 32, 64
EPS = 1e-5


def _cs(num, den):
    a = 2 * np.pi * num / den
    return float(np.cos(a)), float(np.sin(a))


def _dft_real(xs):
    N = len(xs)
    if N == 4:
        c1, s1 = _cs(1, 16); c2 = float(np.sqrt(0.5)); c3, s3 = _cs(3, 16)
        x0, x1, x2, x3 = xs
        y1r, y1i = x1 * c1, x1 * s1
        t2 = x2 * c2
        y3r, y3i = x3 * c3, x3 * s3
        ar = x0 + t2
        br = x0 - t2
        cr, ci = y1r + y3r, y1i + y3i
        dr, di = y1r - y3r, y1i - y3i
        return [(ar + cr, t2 + ci), (br + di, -(t2 + dr)), (ar - cr, t2 - ci), (br - di, dr - t2)]
    if N == 8:
        E = _dft_real(xs[0::2]); O = _dft_real(xs[1::2])
        out = [None] * 8
        for f in range(4):
            c, s = _cs(-(4 * f - 1), 4 * N)
            a, b = O[f]
            tr, ti = a * c - b * s, a * s + b * c
            out[f] = (E[f][0] + tr, E[f][1] + ti)
            out[f + 4] = (E[f][0] - tr, E[f][1] - ti)
        return out
    Q = [_dft_real(xs[p::4]) for p in range(4)]
    n4 = N // 4
    out = [None] * N
    for f in range(n4):
        y = [Q[0][f]]
        for p in range(1, 4):
            c, s = _cs(-p * (4 * f - 1), 4 * N)
            a, b = Q[p][f]
            y.append((a * c - b * s, a * s + b * c))
        ar, ai = y[0][0] + y[2][0], y[0][1] + y[2][1]
        br, bi = y[0][0] - y[2][0], y[0][1] - y[2][1]
        cr, ci = y[1][0] + y[3][0], y[1][1] + y[3][1]
        dr, di = y[1][0] - y[3][0], y[1][1] - y[3][1]
        out[f] = (ar + cr, ai + ci)
        out[f + 2 * n4] = (ar - cr, ai - ci)
        out[f + n4] = (br + di, bi - dr)
        out[f + 3 * n4] = (br - di, bi + dr)
    return out


def _idft_real(B):
    N = len(B)
    if N == 4:
        (a0r, a0i), (a1r, a1i), (a2r, a2i), (a3r, a3i) = B
        ar = a0r + a2r; cr = a0r - a2r
        ai = a0i + a2i; ci = a0i - a2i
        br = a1r + a3r; di = a1r - a3r
        dr = a3i - a1i; m = a1i + a3i
        c1, s1 = _cs(1, 16); c2 = float(np.sqrt(0.5)); c3, s3 = _cs(3, 16)
        y1r, y3r = cr + dr, cr - dr
        y1i, y3i = ci + di, ci - di
        return [ar + br, y1r * c1 + y1i * s1, ((ar - br) + (ai - m)) * c2, y3r * c3 + y3i * s3]
    if N == 8:
        E = [None] * 4; O = [None] * 4
        for f in range(4):
            c, s = _cs(-(4 * f - 1), 4 * N)
            E[f] = (B[f][0] + B[f + 4][0], B[f][1] + B[f + 4][1])
            tr, ti = B[f][0] - B[f + 4][0], B[f][1] - B[f + 4][1]
            O[f] = (tr * c + ti * s, ti * c - tr * s)
        out = [None] * 8
        out[0::2] = _idft_real(E); out[1::2] = _idft_real(O)
        return out
    n4 = N // 4
    Q = [[None] * n4 for _ in range(4)]
    for f in range(n4):
        o0, o1, o2, o3 = B[f], B[f + n4], B[f + 2 * n4], B[f + 3 * n4]
        ar, ai = o0[0] + o2[0], o0[1] + o2[1]
        cr, ci = o0[0] - o2[0], o0[1] - o2[1]
        br, bi = o1[0] + o3[0], o1[1] + o3[1]
        di, dr = o1[0] - o3[0], o3[1] - o1[1]
        y = [(ar + br, ai + bi), (cr + dr, ci + di), (ar - br, ai - bi), (cr - dr, ci - di)]
        Q[0][f] = y[0]
        for p in range(1, 4):
            c, s = _cs(-p * (4 * f - 1), 4 * N)
            a, b = y[p]
            Q[p][f] = (a * c + b * s, b * c - a * s)
    out = [None] * N
    for p in range(4):
        out[p::4] = _idft_real(Q[p])
    return out


def _stage2_tables():
    f1 = np.arange(N1)[:, None, None]
    f2 = np.arange(N2)[None, :, None]
    n2 = np.arange(N2)[None, None, :]
    ph = -2 * np.pi * (n2 * (f1 - 0.25) / S + n2 * f2 / N2)
    gr, gi = np.cos(ph), np.sin(ph)
    g = np.concatenate([np.concatenate([gr, -gi], 2), np.concatenate([gi, gr], 2)], 1)
    perm = np.arange(2 * N2).reshape(2, N2 // 8, 8).transpose(1, 0, 2).reshape(-1)
    g = g[:, :, perm]
    ginv = np.transpose(g, (0, 2, 1)) / S
    return g.astype(jnp.bfloat16), np.ascontiguousarray(ginv).astype(jnp.bfloat16)


_G_FWD, _G_INV = _stage2_tables()


def _ln(x):
    m = jnp.mean(x, axis=-1, keepdims=True)
    xc = x - m
    v = jnp.mean(xc * xc, axis=-1, keepdims=True)
    return xc * jax.lax.rsqrt(v + EPS)


def _gelu(x):
    c = float(np.sqrt(2.0 / np.pi))
    u = x * (c + (c * 0.044715) * (x * x))
    return (0.5 * x) * (1.0 + jnp.tanh(u))


RB = 256
NB = S // RB
SB = 256
U32 = jnp.uint32


def _unp(x):
    return pltpu.bitcast(x, jnp.bfloat16)


def _pk(x):
    return pltpu.bitcast(x.astype(jnp.bfloat16), U32)


def _kernel(q_hbm, k_hbm, v_hbm, sh_ref, ssmk_hbm, d_ref, win_hbm, wsp_hbm, b_ref, wout_hbm,
            g_hbm, gi_hbm, o_hbm,
            q_s, k_s, v_s, ssmk_s, win_s, wsp_s, wout_s, g_s, gi_s, o_s,
            xn_s, z1_s, z2_s, h_s, kv_s, kt_s, ax_s, ak_s, b_s, y_s, bcol_s,
            sem_q, sem_k, sem_v, sem_sk, sem_wsp, sem_o, sem_m):
    f32, bf16 = jnp.float32, jnp.bfloat16
    q_hbm, k_hbm, v_hbm, ssmk_hbm, win_hbm, wsp_hbm, wout_hbm, g_hbm, gi_hbm, o_hbm = (
        r.bitcast(U32) for r in
        (q_hbm, k_hbm, v_hbm, ssmk_hbm, win_hbm, wsp_hbm, wout_hbm, g_hbm, gi_hbm, o_hbm))

    def rows(i, n=RB):
        return pl.ds(pl.multiple_of(i * n, n), n)

    def hrows(i, n=RB):
        return rows(i, n // 2)

    def cp_q(i): return pltpu.make_async_copy(q_hbm.at[hrows(i)], q_s.at[hrows(i)], sem_q.at[i])
    def cp_k(i): return pltpu.make_async_copy(k_hbm.at[hrows(i)], k_s.at[pl.ds(pl.multiple_of(8 + i * (RB // 2), 8), RB // 2)], sem_k.at[i])
    def cp_v(i): return pltpu.make_async_copy(v_hbm.at[hrows(i)], v_s.at[hrows(i)], sem_v.at[i])
    def cp_sk(i): return pltpu.make_async_copy(ssmk_hbm.at[:, rows(i)], ssmk_s.at[:, rows(i)], sem_sk.at[i])
    def cp_wsp(i): return pltpu.make_async_copy(wsp_hbm.at[hrows(i, SB)], wsp_s.at[hrows(i, SB)], sem_wsp.at[i])
    def cp_o(i): return pltpu.make_async_copy(o_s.at[hrows(i)], o_hbm.at[hrows(i)], sem_o.at[i])
    cp_win = pltpu.make_async_copy(win_hbm, win_s, sem_m.at[0])
    cp_wout = pltpu.make_async_copy(wout_hbm, wout_s, sem_m.at[1])
    cp_g = pltpu.make_async_copy(g_hbm, g_s, sem_m.at[2])
    cp_gi = pltpu.make_async_copy(gi_hbm, gi_s, sem_m.at[3])

    def start_a(i):
        cp_q(i).start(); cp_k(i).start(); cp_v(i).start(); cp_sk(i).start()

    cp_q(0).start(); cp_win.start()
    cp_k(0).start(); cp_v(0).start(); cp_sk(0).start()

    sh = sh_ref[...].astype(f32)
    dvec = d_ref[...].astype(f32).reshape(1, D)
    bcol_s[...] = jnp.broadcast_to(b_ref[...].astype(f32).reshape(1, S), (128, S)).T
    k_s[0:8, :] = jnp.zeros((8, D), U32)
    cp_win.wait()
    start_a(1)

    def loop_a(i, carry):
        r, hr = rows(i), hrows(i)
        @pl.when(i + 2 < NB)
        def _():
            start_a(i + 2)
        @pl.when(i + 2 >= NB)
        def _():
            j = 2 * (i + 2 - NB)
            cp_wsp(j).start(); cp_wsp(j + 1).start()
        cp_q(i).wait(); cp_k(i).wait(); cp_v(i).wait(); cp_sk(i).wait()
        xn = _ln(_unp(q_s[hr, :]).astype(f32)).astype(bf16)
        xn_s[hr, :] = _pk(xn)
        z2 = _gelu(jnp.dot(xn, _unp(win_s[:, FH:]), preferred_element_type=f32))
        z2_s[hr, :] = _pk(_ln(z2))
        z1_s[hr, :] = _pk(_gelu(jnp.dot(xn, _unp(win_s[:, :FH]), preferred_element_type=f32)))
        for c in range(D // 128):
            cs = slice(c * 128, (c + 1) * 128)
            kt_s[r, cs] = _unp(ssmk_s[c * 64:(c + 1) * 64, r]).astype(f32).T
            kk = _unp(k_s[pl.ds(pl.multiple_of(i * (RB // 2), 8), RB // 2 + 8), cs]).astype(f32)
            kk = kk[8:]
            acc = kk[8:] * sh[0:1, cs]
            for t in range(1, 4):
                acc = acc + pltpu.roll(kk, t, 0)[8:] * sh[t:t + 1, cs]
            kv_s[r, cs] = acc * _unp(v_s[hr, cs]).astype(f32)
        return carry
    with jax.named_scope('A'):
        jax.lax.fori_loop(0, NB, loop_a, 0)

    def spatial(i):
        r, hr = rows(i, SB), hrows(i, SB)
        cp_wsp(i).wait()
        g = jnp.dot(_unp(wsp_s[hr, :]), _unp(z2_s[...]), preferred_element_type=f32)
        g = g + jnp.concatenate([bcol_s[r, :]] * (FH // 128), axis=1)
        h_s[hr, :] = _pk(_unp(z1_s[hr, :]).astype(f32) * g)

    nsb = S // SB // 2
    cp_g.start(); cp_gi.start()
    for j in range(nsb, 2 * nsb):
        cp_wsp(j).start()
    cp_wout.start()

    def loop_b(i, carry):
        spatial(i)
        per = 8 // nsb
        for u in range(per):
            r0 = pl.multiple_of((i * per + u) * 8, 8)
            for c in range(D // 128):
                cs = slice(c * 128, (c + 1) * 128)
                for src, dst in ((kv_s, ax_s), (kt_s, ak_s)):
                    res = _dft_real([src[pl.ds(n1 * N2 + r0, 8), cs] for n1 in range(N1)])
                    for f in range(N1):
                        dst[f, pl.ds(r0, 8), cs] = _pk(jnp.concatenate(res[f], 0))
        return carry
    with jax.named_scope('B'):
        jax.lax.fori_loop(0, nsb, loop_b, 0)

    cp_g.wait(); cp_gi.wait()
    def loop_c(i, carry):
        for u in range(4):
            f = i * 4 + u
            gf = _unp(g_s[f])
            X = jnp.dot(gf, _unp(ax_s[f]), preferred_element_type=f32)
            K = jnp.dot(gf, _unp(ak_s[f]), preferred_element_type=f32)
            xr, xi, kr, ki = X[:N2], X[N2:], K[:N2], K[N2:]
            Y = jnp.concatenate([xr * kr - xi * ki, xr * ki + xi * kr], 0).astype(bf16)
            b_s[f] = jnp.dot(_unp(gi_s[f]), Y, preferred_element_type=f32)
        return carry
    with jax.named_scope('C'):
        jax.lax.fori_loop(0, N1 // 4, loop_c, 0)

    def loop_d(i, carry):
        spatial(i + nsb)
        per = 4 // nsb
        for u in range(per):
            g = i * per + u
            for c in range(D // 128):
                cs = slice(c * 128, (c + 1) * 128)
                ys = []
                for h in range(2):
                    rb = pl.multiple_of(g * 32 + h * 16, 16)
                    ys.append(_idft_real([(b_s[f, pl.ds(rb, 8), cs], b_s[f, pl.ds(rb + 8, 8), cs]) for f in range(N1)]))
                for n1 in range(N1):
                    y_s[pl.ds(pl.multiple_of(n1 * (N2 // 2) + g * 8, 8), 8), cs] = _pk(jnp.concatenate([ys[0][n1], ys[1][n1]], 0))
        return carry
    with jax.named_scope('D'):
        jax.lax.fori_loop(0, nsb, loop_d, 0)

    cp_wout.wait()
    def loop_e(i, carry):
        r, hr = rows(i), hrows(i)
        o = jnp.dot(_unp(h_s[hr, :]), _unp(wout_s[...]), preferred_element_type=f32)
        gate = o / (1.0 + jnp.exp(-o))
        y = _unp(y_s[hr, :]).astype(f32) + kv_s[r, :] * dvec
        o_s[hr, :] = _pk(_unp(q_s[hr, :]).astype(f32) + _unp(xn_s[hr, :]).astype(f32) * y * gate)
        cp_o(i).start()
        return carry
    with jax.named_scope('E'):
        jax.lax.fori_loop(0, NB, loop_e, 0)
    for i in range(NB):
        cp_o(i).wait()


@jax.jit
def pallas_recurrent_scan__ssm_conv_h3__mixer_gmlp__prompt_kernel(
    A_q: jax.Array,
    A_k: jax.Array,
    A_v: jax.Array,
    A_shift_k: jax.Array,
    A_ssm_k: jax.Array,
    A_ssm_D: jax.Array,
    B_x: jax.Array,
    B_w_in: jax.Array,
    B_w_sp: jax.Array,
    B_b_sp: jax.Array,
    B_w_out: jax.Array,
):
    del B_x
    f32 = jnp.float32
    hbm = pl.BlockSpec(memory_space=pl.ANY)
    vm = pl.BlockSpec(memory_space=pltpu.VMEM)
    out = pl.pallas_call(
        _kernel,
        out_shape=jax.ShapeDtypeStruct((S, D), A_q.dtype),
        in_specs=[hbm, hbm, hbm, vm, hbm, vm, hbm, hbm, vm, hbm, hbm, hbm],
        out_specs=hbm,
        scratch_shapes=[
            pltpu.VMEM((S // 2, D), U32),
            pltpu.VMEM((S // 2 + 8, D), U32),
            pltpu.VMEM((S // 2, D), U32),
            pltpu.VMEM((D // 2, S), U32),
            pltpu.VMEM((D // 2, F), U32),
            pltpu.VMEM((S // 2, S), U32),
            pltpu.VMEM((FH // 2, D), U32),
            pltpu.VMEM((N1, N2, 2 * N2), U32),
            pltpu.VMEM((N1, N2, 2 * N2), U32),
            pltpu.VMEM((S // 2, D), U32),
            pltpu.VMEM((S // 2, D), U32),
            pltpu.VMEM((S // 2, FH), U32),
            pltpu.VMEM((S // 2, FH), U32),
            pltpu.VMEM((S // 2, FH), U32),
            pltpu.VMEM((S, D), f32),
            pltpu.VMEM((S, D), f32),
            pltpu.VMEM((N1, N2, D), U32),
            pltpu.VMEM((N1, N2, D), U32),
            pltpu.VMEM((N1, 2 * N2, D), f32),
            pltpu.VMEM((S // 2, D), U32),
            pltpu.VMEM((S, 128), f32),
            pltpu.SemaphoreType.DMA((NB,)),
            pltpu.SemaphoreType.DMA((NB,)),
            pltpu.SemaphoreType.DMA((NB,)),
            pltpu.SemaphoreType.DMA((NB,)),
            pltpu.SemaphoreType.DMA((S // SB,)),
            pltpu.SemaphoreType.DMA((NB,)),
            pltpu.SemaphoreType.DMA((4,)),
        ],
        compiler_params=pltpu.CompilerParams(vmem_limit_bytes=120 << 20),
    )(A_q.reshape(S, D), A_k.reshape(S, D), A_v.reshape(S, D), A_shift_k.T, A_ssm_k,
      A_ssm_D, B_w_in, B_w_sp, B_b_sp, B_w_out, _G_FWD, _G_INV)
    return out.reshape(A_q.shape)
```

```python
import functools
import numpy as np
import jax
import jax.numpy as jnp
import jax.experimental.pallas as pl
import jax.experimental.pallas.tpu as pltpu

S, D, F, FH = 2048, 640, 1536, 768
N1, N2 = 32, 64
EPS = 1e-5


def _cs(num, den):
    a = 2 * np.pi * num / den
    return float(np.cos(a)), float(np.sin(a))


_C1, _S1 = _cs(1, 16)
_C2 = float(np.sqrt(0.5))
_C3, _S3 = _cs(3, 16)


def _rot(a, b, c, s):
    return a * c - b * s, a * s + b * c


def _rot_t(a, b, c, s):
    return a * c + b * s, b * c - a * s


def _dft4(xs, C):
    c1, s1, c2, c3, s3 = C
    x0, x1, x2, x3 = xs
    y1r, y1i = x1 * c1, x1 * s1
    t2 = x2 * c2
    y3r, y3i = x3 * c3, x3 * s3
    ar, br = x0 + t2, x0 - t2
    cr, ci = y1r + y3r, y1i + y3i
    dr, di = y1r - y3r, y1i - y3i
    return [(ar + cr, t2 + ci), (br + di, -(t2 + dr)), (ar - cr, t2 - ci), (br - di, dr - t2)]


def _dft8(xs, gc):
    C = [gc(c) for c in (_C1, _S1, _C2, _C3, _S3)]
    E, O = _dft4(xs[0::2], C), _dft4(xs[1::2], C)
    out = [None] * 8
    for f in range(4):
        tr, ti = _rot(*O[f], *_cs(-(4 * f - 1), 32))
        out[f] = (E[f][0] + tr, E[f][1] + ti)
        out[f + 4] = (E[f][0] - tr, E[f][1] - ti)
    return out


def _radix4(Q, f, gc):
    y = [Q[0]]
    for p in range(1, 4):
        c, s = _cs(-p * (4 * f - 1), 4 * N1)
        y.append(_rot(*Q[p], gc(c), gc(s)))
    ar, ai = y[0][0] + y[2][0], y[0][1] + y[2][1]
    br, bi = y[0][0] - y[2][0], y[0][1] - y[2][1]
    cr, ci = y[1][0] + y[3][0], y[1][1] + y[3][1]
    dr, di = y[1][0] - y[3][0], y[1][1] - y[3][1]
    return [(ar + cr, ai + ci), (br + di, bi - dr), (ar - cr, ai - ci), (br - di, bi + dr)]


def _radix4_t(o, f):
    o0, o1, o2, o3 = o
    ar, ai = o0[0] + o2[0], o0[1] + o2[1]
    cr, ci = o0[0] - o2[0], o0[1] - o2[1]
    br, bi = o1[0] + o3[0], o1[1] + o3[1]
    di, dr = o1[0] - o3[0], o3[1] - o1[1]
    y = [(ar + br, ai + bi), (cr + dr, ci + di), (ar - br, ai - bi), (cr - dr, ci - di)]
    return [y[0]] + [_rot_t(*y[p], *_cs(-p * (4 * f - 1), 4 * N1)) for p in range(1, 4)]


def _dft4_t(B):
    (a0r, a0i), (a1r, a1i), (a2r, a2i), (a3r, a3i) = B
    ar, cr = a0r + a2r, a0r - a2r
    ai, ci = a0i + a2i, a0i - a2i
    br, di = a1r + a3r, a1r - a3r
    dr, m = a3i - a1i, a1i + a3i
    return [ar + br, (cr + dr) * _C1 + (ci + di) * _S1, ((ar - br) + (ai - m)) * _C2, (cr - dr) * _C3 + (ci - di) * _S3]


def _dft8_t(B):
    E, O = [None] * 4, [None] * 4
    for f in range(4):
        E[f] = (B[f][0] + B[f + 4][0], B[f][1] + B[f + 4][1])
        O[f] = _rot_t(B[f][0] - B[f + 4][0], B[f][1] - B[f + 4][1], *_cs(-(4 * f - 1), 32))
    out = [None] * 8
    out[0::2] = _dft4_t(E)
    out[1::2] = _dft4_t(O)
    return out


def _stage2_tables():
    f1 = np.arange(N1)[:, None, None]
    f2 = np.arange(N2)[None, :, None]
    n2 = np.arange(N2)[None, None, :]
    ph = -2 * np.pi * (n2 * (f1 - 0.25) / S + n2 * f2 / N2)
    gr, gi = np.cos(ph), np.sin(ph)
    g = np.concatenate([np.concatenate([gr, -gi], 2), np.concatenate([gi, gr], 2)], 1)
    perm = np.arange(2 * N2).reshape(2, N2 // 8, 8).transpose(1, 0, 2).reshape(-1)
    g = g[:, :, perm]
    ginv = np.transpose(g, (0, 2, 1)) / S
    return g.astype(jnp.bfloat16), np.ascontiguousarray(ginv).astype(jnp.bfloat16)


_G_FWD, _G_INV = _stage2_tables()


def _ln(x):
    m = jnp.mean(x, axis=-1, keepdims=True)
    xc = x - m
    v = jnp.mean(xc * xc, axis=-1, keepdims=True)
    return xc * jax.lax.rsqrt(v + EPS)


def _gelu(x):
    c = float(np.sqrt(2.0 / np.pi))
    u = x * (c + (c * 0.044715) * (x * x))
    return (0.5 * x) * (1.0 + jnp.tanh(u))


RB = 256
NB = S // RB
SB = RB
MA = 256
KV = 32
KC = 256
U32 = jnp.uint32


def _unp(x):
    return pltpu.bitcast(x, jnp.bfloat16)


def _pk(x):
    return pltpu.bitcast(x.astype(jnp.bfloat16), U32)


def _kernel(q_hbm, k_hbm, v_hbm, sh_ref, ssmk_hbm, d_ref, win_hbm, wsp_hbm, b_ref, wout_hbm,
            g_hbm, gi_hbm, o_hbm,
            q_s, k_s, v_s, ssmk_s, win_s, wsp_s, wout_s, g_s, gi_s, o_s,
            xn_s, z1_s, z2_s, h_s, kv_s, kt_s, ax_s, ak_s, b_s, y_s, bcol_s, z2f_s, t_s,
            sem_q, sem_k, sem_v, sem_sk, sem_wsp, sem_o, sem_m):
    f32, bf16 = jnp.float32, jnp.bfloat16
    q_hbm, k_hbm, v_hbm, ssmk_hbm, win_hbm, wsp_hbm, wout_hbm, g_hbm, gi_hbm, o_hbm = (
        r.bitcast(U32) for r in
        (q_hbm, k_hbm, v_hbm, ssmk_hbm, win_hbm, wsp_hbm, wout_hbm, g_hbm, gi_hbm, o_hbm))

    def rows(i, n=RB):
        return pl.ds(pl.multiple_of(i * n, n), n)

    def hrows(i, n=RB):
        return rows(i, n // 2)

    def cp_q(i): return pltpu.make_async_copy(q_hbm.at[hrows(i)], q_s.at[hrows(i)], sem_q.at[i])
    def cp_k(i): return pltpu.make_async_copy(k_hbm.at[hrows(i)], k_s.at[pl.ds(pl.multiple_of(8 + i * (RB // 2), 8), RB // 2)], sem_k.at[i])
    def cp_v(i): return pltpu.make_async_copy(v_hbm.at[hrows(i)], v_s.at[hrows(i)], sem_v.at[i])
    def cp_sk(i): return pltpu.make_async_copy(ssmk_hbm.at[:, rows(i)], ssmk_s.at[:, rows(i)], sem_sk.at[i])
    def cp_wsp(i): return pltpu.make_async_copy(wsp_hbm.at[hrows(i, SB)], wsp_s.at[hrows(i, SB)], sem_wsp.at[i])
    def cp_o(i): return pltpu.make_async_copy(o_s.at[hrows(i)], o_hbm.at[hrows(i)], sem_o.at[i])
    cp_win = pltpu.make_async_copy(win_hbm, win_s, sem_m.at[0])
    cp_wout = pltpu.make_async_copy(wout_hbm, wout_s, sem_m.at[1])
    cp_g = pltpu.make_async_copy(g_hbm, g_s, sem_m.at[2])
    cp_gi = pltpu.make_async_copy(gi_hbm, gi_s, sem_m.at[3])

    cp_q(0).start(); cp_q(1).start(); cp_win.start()
    cp_k(0).start(); cp_v(0).start(); cp_sk(0).start()

    sh = sh_ref[...].astype(f32)
    dvec = d_ref[...].astype(f32).reshape(1, D)
    bcol_s[...] = jnp.broadcast_to(b_ref[...].astype(f32).reshape(1, S), (128, S)).T
    k_s[0:8, :] = jnp.zeros((8, D), U32)

    def run(steps, pieces):
        for s_, step in enumerate(steps):
            acc = step()
            never = acc[0:8, 0:128] > jnp.inf
            lo, hi = s_ * len(pieces) // len(steps), (s_ + 1) * len(pieces) // len(steps)
            for piece in pieces[lo:hi]:
                piece(lambda c: jnp.where(jnp.broadcast_to(never[0:1], c.shape) if hasattr(c, 'shape') and c.shape != (8, 128) else never, 0.0 if not hasattr(c, 'dtype') else jnp.zeros_like(c), c))

    def lanes(c):
        return slice(c * 128, (c + 1) * 128)

    def xn_piece(j, g, gc=None):
        hr = pl.ds(pl.multiple_of(j * (RB // 2) + g * 8, 8), 8)
        x = q_s[hr, :]
        if gc is not None:
            x = jnp.concatenate([x[:, lanes(c)] for c in range(D // 128)], 1)
        x = _unp(x).astype(f32)
        xn_s[hr, :] = _pk(_ln(x))

    cp_q(0).wait()
    for g in range(RB // 16):
        xn_piece(0, g)
    cp_win.wait()
    cp_k(1).start(); cp_v(1).start(); cp_sk(1).start(); cp_q(2).start()

    def loop_a(i, carry):
        r, hr = rows(i), hrows(i)
        @pl.when(i + 2 < NB)
        def _():
            cp_k(i + 2).start(); cp_v(i + 2).start(); cp_sk(i + 2).start()
        @pl.when(i + 3 < NB)
        def _():
            cp_q(i + 3).start()
        @pl.when(i + 3 >= NB)
        def _():
            cp_wsp(i + 3 - NB).start()
        @pl.when(i + 1 < NB)
        def _():
            cp_q(i + 1).wait()
        cp_k(i).wait(); cp_v(i).wait(); cp_sk(i).wait()
        nxt = jnp.minimum(i + 1, NB - 1)

        def step(n, m):
            def f():
                hm = pl.ds(pl.multiple_of(i * (RB // 2) + m * (MA // 2), 8), MA // 2)
                d = jnp.dot(_unp(xn_s[hm, :]), _unp(win_s[:, lanes(n)]), preferred_element_type=f32)
                z = _gelu(d)
                if n < FH // 128:
                    z1_s[hm, lanes(n)] = _pk(z)
                else:
                    z2f_s[m * MA:(m + 1) * MA, lanes(n - FH // 128)] = z
                return d
            return f

        def ln_piece(g):
            def f(gc):
                z = jnp.concatenate([z2f_s[g * 16:(g + 1) * 16, lanes(c)] for c in range(FH // 128)], 1)
                z2_s[pl.ds(pl.multiple_of(i * (RB // 2) + g * 8, 8), 8), :] = _pk(_ln(z))
            return f

        def kv_piece(c, g):
            def f(gc):
                h0 = pl.multiple_of(i * (RB // 2) + g * (KV // 2), 8)
                kk = _unp(gc(k_s[pl.ds(h0, KV // 2 + 8), lanes(c)])).astype(f32)[8:]
                w = [sh[t:t + 1, lanes(c)] for t in range(4)]
                acc = kk[8:] * w[0]
                for t in range(1, 4):
                    acc = acc + pltpu.roll(kk, t, 0)[8:] * w[t]
                kv_s[pl.ds(pl.multiple_of(i * RB + g * KV, 8), KV), lanes(c)] = acc * _unp(v_s[pl.ds(h0, KV // 2), lanes(c)]).astype(f32)
            return f

        def kt_piece(c, g):
            def f(gc):
                t0 = pl.ds(pl.multiple_of(i * RB + g * 128, 128), 128)
                kt_s[t0, lanes(c)] = _unp(ssmk_s[c * 64:(c + 1) * 64, t0]).astype(f32).T
            return f

        nt = FH // 128
        early = [kv_piece(c, g) for c in range(D // 128) for g in range(RB // KV)]
        early += [kt_piece(c, g) for c in range(D // 128) for g in range(RB // 128)]
        late = [ln_piece(g) for g in range(RB // 16)]
        late += [functools.partial(xn_piece, nxt, g) for g in range(RB // 16)]
        run([step(n, m) for n in range(nt, 2 * nt) for m in range(RB // MA)], early)
        run([step(n, m) for n in range(nt) for m in range(RB // MA)], late)
        return carry
    jax.lax.fori_loop(0, NB, loop_a, 0)

    def spatial_steps(i, tiles):
        r, hr = rows(i), hrows(i)
        steps = []
        for n in tiles:
            box = [None]
            hn = hrows(jnp.minimum(i, NB + n))
            for k in range(S // KC):
                def f(n=n, k=k, box=box, hn=hn):
                    d = jnp.dot(_unp(wsp_s[hn, k * KC:(k + 1) * KC]), _unp(z2_s[k * KC // 2:(k + 1) * KC // 2, lanes(n)]),
                                preferred_element_type=f32)
                    box[0] = d if k == 0 else box[0] + d
                    if k == S // KC - 1:
                        h_s[hr, lanes(n)] = _pk(_unp(z1_s[hr, lanes(n)]).astype(f32) * (box[0] + bcol_s[r, :]))
                    return box[0]
                steps.append(f)
        return steps

    cp_g.start(); cp_gi.start()

    def loop_b(i, carry):
        @pl.when(i + 3 < NB)
        def _():
            cp_wsp(i + 3).start()
        @pl.when(i + 3 == NB)
        def _():
            cp_wout.start()
        cp_wsp(i).wait()
        r0 = pl.multiple_of(i * 8, 8)
        pieces = []
        for u, (src, dst) in enumerate(((kv_s, ax_s), (kt_s, ak_s)) * (D // 128)):
            c = u // 2
            def p1(p, u=u, c=c, src=src):
                def f(gc):
                    Q = _dft8([src[pl.ds((4 * m + p) * N2 + r0, 8), lanes(c)] for m in range(8)], gc)
                    for q in range(8):
                        t_s[u % 2, p * 8 + q, 0:8, :] = Q[q][0]
                        t_s[u % 2, p * 8 + q, 8:16, :] = Q[q][1]
                return f
            def p2(q, u=u, c=c, dst=dst):
                def f(gc):
                    o = _radix4([(t_s[u % 2, p * 8 + q, 0:8, :], t_s[u % 2, p * 8 + q, 8:16, :]) for p in range(4)], q, gc)
                    for j in range(4):
                        dst[q + 8 * j, pl.ds(r0, 8), lanes(c)] = _pk(jnp.concatenate(o[j], 0))
                return f
            pieces += [p1(p) for p in range(4)] + [p2(q) for q in range(8)]
        run(spatial_steps(i, (0, 1, 2)), pieces)
        return carry
    jax.lax.fori_loop(0, NB, loop_b, 0)

    cp_g.wait(); cp_gi.wait()

    def loop_c(i, carry):
        sp = spatial_steps(i, (3,))
        for u in range(4):
            f = i * 4 + u
            gf = _unp(g_s[f])
            X = jnp.dot(gf, _unp(ax_s[f]), preferred_element_type=f32)
            K = jnp.dot(gf, _unp(ak_s[f]), preferred_element_type=f32)
            for st in sp[u * len(sp) // 4:(u + 1) * len(sp) // 4]:
                st()
            xr, xi, kr, ki = X[:N2], X[N2:], K[:N2], K[N2:]
            Y = jnp.concatenate([xr * kr - xi * ki, xr * ki + xi * kr], 0).astype(bf16)
            b_s[f] = jnp.dot(_unp(gi_s[f]), Y, preferred_element_type=f32)
        return carry
    jax.lax.fori_loop(0, NB, loop_c, 0)

    def loop_d(i, carry):
        rb = pl.multiple_of(i * 16, 16)
        pieces = []
        for c in range(D // 128):
            def p1(q, c=c):
                def f(gc):
                    z = gc(0.0)
                    o = _radix4_t([(b_s[q + 8 * j, pl.ds(rb, 8), lanes(c)] + z, b_s[q + 8 * j, pl.ds(rb + 8, 8), lanes(c)] + z)
                                   for j in range(4)], q)
                    for p in range(4):
                        t_s[c % 2, p * 8 + q, 0:8, :] = o[p][0]
                        t_s[c % 2, p * 8 + q, 8:16, :] = o[p][1]
                return f
            def p2(p, c=c):
                def f(gc):
                    z = gc(0.0)
                    y = _dft8_t([(t_s[c % 2, p * 8 + q, 0:8, :] + z, t_s[c % 2, p * 8 + q, 8:16, :] + z) for q in range(8)])
                    for m in range(8):
                        y_s[pl.ds(pl.multiple_of((4 * m + p) * N2 + i * 8, 8), 8), lanes(c)] = y[m]
                return f
            pieces += [p1(q) for q in range(8)] + [p2(p) for p in range(4)]
        run(spatial_steps(i, (4, 5)), pieces)
        return carry
    jax.lax.fori_loop(0, NB, loop_d, 0)

    cp_wout.wait()

    def loop_e(i, carry):
        r, hr = rows(i), hrows(i)
        o = jnp.dot(_unp(h_s[hr, :]), _unp(wout_s[...]), preferred_element_type=f32)
        ho = 0.5 * o
        gate = ho * jnp.tanh(ho) + ho
        y = y_s[r, :] + kv_s[r, :] * dvec
        o_s[hr, :] = _pk(_unp(q_s[hr, :]).astype(f32) + _unp(xn_s[hr, :]).astype(f32) * y * gate)
        cp_o(i).start()
        return carry
    jax.lax.fori_loop(0, NB, loop_e, 0)
    for i in range(NB):
        cp_o(i).wait()


@jax.jit
def pallas_recurrent_scan__ssm_conv_h3__mixer_gmlp__prompt_kernel(
    A_q: jax.Array,
    A_k: jax.Array,
    A_v: jax.Array,
    A_shift_k: jax.Array,
    A_ssm_k: jax.Array,
    A_ssm_D: jax.Array,
    B_x: jax.Array,
    B_w_in: jax.Array,
    B_w_sp: jax.Array,
    B_b_sp: jax.Array,
    B_w_out: jax.Array,
):
    del B_x
    f32 = jnp.float32
    hbm = pl.BlockSpec(memory_space=pl.ANY)
    vm = pl.BlockSpec(memory_space=pltpu.VMEM)
    out = pl.pallas_call(
        _kernel,
        out_shape=jax.ShapeDtypeStruct((S, D), A_q.dtype),
        in_specs=[hbm, hbm, hbm, vm, hbm, vm, hbm, hbm, vm, hbm, hbm, hbm],
        out_specs=hbm,
        scratch_shapes=[
            pltpu.VMEM((S // 2, D), U32),
            pltpu.VMEM((S // 2 + 8, D), U32),
            pltpu.VMEM((S // 2, D), U32),
            pltpu.VMEM((D // 2, S), U32),
            pltpu.VMEM((D // 2, F), U32),
            pltpu.VMEM((S // 2, S), U32),
            pltpu.VMEM((FH // 2, D), U32),
            pltpu.VMEM((N1, N2, 2 * N2), U32),
            pltpu.VMEM((N1, N2, 2 * N2), U32),
            pltpu.VMEM((S // 2, D), U32),
            pltpu.VMEM((S // 2, D), U32),
            pltpu.VMEM((S // 2, FH), U32),
            pltpu.VMEM((S // 2, FH), U32),
            pltpu.VMEM((S // 2, FH), U32),
            pltpu.VMEM((S, D), f32),
            pltpu.VMEM((S, D), f32),
            pltpu.VMEM((N1, N2, D), U32),
            pltpu.VMEM((N1, N2, D), U32),
            pltpu.VMEM((N1, 2 * N2, D), f32),
            pltpu.VMEM((S, D), f32),
            pltpu.VMEM((S, 128), f32),
            pltpu.VMEM((RB, FH), f32),
            pltpu.VMEM((10, N1, 16, 128), f32),
            pltpu.SemaphoreType.DMA((NB,)),
            pltpu.SemaphoreType.DMA((NB,)),
            pltpu.SemaphoreType.DMA((NB,)),
            pltpu.SemaphoreType.DMA((NB,)),
            pltpu.SemaphoreType.DMA((S // SB,)),
            pltpu.SemaphoreType.DMA((NB,)),
            pltpu.SemaphoreType.DMA((4,)),
        ],
        compiler_params=pltpu.CompilerParams(vmem_limit_bytes=120 << 20),
    )(A_q.reshape(S, D), A_k.reshape(S, D), A_v.reshape(S, D), A_shift_k.T, A_ssm_k,
      A_ssm_D, B_w_in, B_w_sp, B_b_sp, B_w_out, _G_FWD, _G_INV)
    return out.reshape(A_q.shape)
```

```python
import functools
import numpy as np
import jax
import jax.numpy as jnp
import jax.experimental.pallas as pl
import jax.experimental.pallas.tpu as pltpu

S, D, F, FH = 2048, 640, 1536, 768
N1, N2 = 32, 64
EPS = 1e-5


def _cs(num, den):
    a = 2 * np.pi * num / den
    return float(np.cos(a)), float(np.sin(a))


_C1, _S1 = _cs(1, 16)
_C2 = float(np.sqrt(0.5))
_C3, _S3 = _cs(3, 16)


def _rot(a, b, c, s):
    return a * c - b * s, a * s + b * c


def _rot_t(a, b, c, s):
    return a * c + b * s, b * c - a * s


def _dft4(xs, C):
    c1, s1, c2, c3, s3 = C
    x0, x1, x2, x3 = xs
    y1r, y1i = x1 * c1, x1 * s1
    t2 = x2 * c2
    y3r, y3i = x3 * c3, x3 * s3
    ar, br = x0 + t2, x0 - t2
    cr, ci = y1r + y3r, y1i + y3i
    dr, di = y1r - y3r, y1i - y3i
    return [(ar + cr, t2 + ci), (br + di, -(t2 + dr)), (ar - cr, t2 - ci), (br - di, dr - t2)]


def _dft8(xs, gc):
    C = [gc(c) for c in (_C1, _S1, _C2, _C3, _S3)]
    E, O = _dft4(xs[0::2], C), _dft4(xs[1::2], C)
    out = [None] * 8
    for f in range(4):
        tr, ti = _rot(*O[f], *_cs(-(4 * f - 1), 32))
        out[f] = (E[f][0] + tr, E[f][1] + ti)
        out[f + 4] = (E[f][0] - tr, E[f][1] - ti)
    return out


def _radix4(Q, f, gc):
    y = [Q[0]]
    for p in range(1, 4):
        c, s = _cs(-p * (4 * f - 1), 4 * N1)
        y.append(_rot(*Q[p], gc(c), gc(s)))
    ar, ai = y[0][0] + y[2][0], y[0][1] + y[2][1]
    br, bi = y[0][0] - y[2][0], y[0][1] - y[2][1]
    cr, ci = y[1][0] + y[3][0], y[1][1] + y[3][1]
    dr, di = y[1][0] - y[3][0], y[1][1] - y[3][1]
    return [(ar + cr, ai + ci), (br + di, bi - dr), (ar - cr, ai - ci), (br - di, bi + dr)]


def _radix4_t(o, f):
    o0, o1, o2, o3 = o
    ar, ai = o0[0] + o2[0], o0[1] + o2[1]
    cr, ci = o0[0] - o2[0], o0[1] - o2[1]
    br, bi = o1[0] + o3[0], o1[1] + o3[1]
    di, dr = o1[0] - o3[0], o3[1] - o1[1]
    y = [(ar + br, ai + bi), (cr + dr, ci + di), (ar - br, ai - bi), (cr - dr, ci - di)]
    return [y[0]] + [_rot_t(*y[p], *_cs(-p * (4 * f - 1), 4 * N1)) for p in range(1, 4)]


def _dft4_t(B):
    (a0r, a0i), (a1r, a1i), (a2r, a2i), (a3r, a3i) = B
    ar, cr = a0r + a2r, a0r - a2r
    ai, ci = a0i + a2i, a0i - a2i
    br, di = a1r + a3r, a1r - a3r
    dr, m = a3i - a1i, a1i + a3i
    return [ar + br, (cr + dr) * _C1 + (ci + di) * _S1, ((ar - br) + (ai - m)) * _C2, (cr - dr) * _C3 + (ci - di) * _S3]


def _dft8_t(B):
    E, O = [None] * 4, [None] * 4
    for f in range(4):
        E[f] = (B[f][0] + B[f + 4][0], B[f][1] + B[f + 4][1])
        O[f] = _rot_t(B[f][0] - B[f + 4][0], B[f][1] - B[f + 4][1], *_cs(-(4 * f - 1), 32))
    out = [None] * 8
    out[0::2] = _dft4_t(E)
    out[1::2] = _dft4_t(O)
    return out


def _stage2_tables():
    f1 = np.arange(N1)[:, None, None]
    f2 = np.arange(N2)[None, :, None]
    n2 = np.arange(N2)[None, None, :]
    ph = -2 * np.pi * (n2 * (f1 - 0.25) / S + n2 * f2 / N2)
    gr, gi = np.cos(ph), np.sin(ph)
    g = np.concatenate([np.concatenate([gr, -gi], 2), np.concatenate([gi, gr], 2)], 1)
    perm = np.arange(2 * N2).reshape(2, N2 // 8, 8).transpose(1, 0, 2).reshape(-1)
    g = g[:, :, perm]
    ginv = np.transpose(g, (0, 2, 1)) / S
    return g.astype(jnp.bfloat16), np.ascontiguousarray(ginv).astype(jnp.bfloat16)


_G_FWD, _G_INV = _stage2_tables()


def _ln(x):
    m = jnp.mean(x, axis=-1, keepdims=True)
    xc = x - m
    v = jnp.mean(xc * xc, axis=-1, keepdims=True)
    return xc * jax.lax.rsqrt(v + EPS)


def _gelu(x):
    c = float(np.sqrt(2.0 / np.pi))
    u = x * (c + (c * 0.044715) * (x * x))
    return (0.5 * x) * (1.0 + jnp.tanh(u))


RB = 256
NB = S // RB
SB = RB
MA = 256
KV = 16
MS = 128
KC = 256
U32 = jnp.uint32


def _unp(x):
    return pltpu.bitcast(x, jnp.bfloat16)


def _pk(x):
    return pltpu.bitcast(x.astype(jnp.bfloat16), U32)


def _kernel(q_hbm, k_hbm, v_hbm, sh_ref, ssmk_hbm, d_ref, win_hbm, wsp_hbm, b_ref, wout_hbm,
            g_hbm, gi_hbm, o_hbm,
            q_s, k_s, v_s, ssmk_s, win_s, wsp_s, wout_s, g_s, gi_s, o_s,
            xn_s, z1_s, z2_s, h_s, kv_s, kt_s, ax_s, ak_s, b_s, y_s, bcol_s, z2f_s, t_s,
            sem_q, sem_k, sem_v, sem_sk, sem_wsp, sem_o, sem_m):
    f32, bf16 = jnp.float32, jnp.bfloat16
    q_hbm, k_hbm, v_hbm, ssmk_hbm, win_hbm, wsp_hbm, wout_hbm, g_hbm, gi_hbm, o_hbm = (
        r.bitcast(U32) for r in
        (q_hbm, k_hbm, v_hbm, ssmk_hbm, win_hbm, wsp_hbm, wout_hbm, g_hbm, gi_hbm, o_hbm))

    def rows(i, n=RB):
        return pl.ds(pl.multiple_of(i * n, n), n)

    def hrows(i, n=RB):
        return rows(i, n // 2)

    def cp_q(i): return pltpu.make_async_copy(q_hbm.at[hrows(i)], q_s.at[hrows(i)], sem_q.at[i])
    def cp_k(i): return pltpu.make_async_copy(k_hbm.at[hrows(i)], k_s.at[pl.ds(pl.multiple_of(8 + i * (RB // 2), 8), RB // 2)], sem_k.at[i])
    def cp_v(i): return pltpu.make_async_copy(v_hbm.at[hrows(i)], v_s.at[hrows(i)], sem_v.at[i])
    def cp_sk(i): return pltpu.make_async_copy(ssmk_hbm.at[:, rows(i)], ssmk_s.at[:, rows(i)], sem_sk.at[i])
    def cp_wsp(i): return pltpu.make_async_copy(wsp_hbm.at[hrows(i, SB)], wsp_s.at[hrows(i, SB)], sem_wsp.at[i])
    def cp_o(i): return pltpu.make_async_copy(o_s.at[hrows(i)], o_hbm.at[hrows(i)], sem_o.at[i])
    cp_win = pltpu.make_async_copy(win_hbm, win_s, sem_m.at[0])
    cp_wout = pltpu.make_async_copy(wout_hbm, wout_s, sem_m.at[1])
    cp_g = pltpu.make_async_copy(g_hbm, g_s, sem_m.at[2])
    cp_gi = pltpu.make_async_copy(gi_hbm, gi_s, sem_m.at[3])

    cp_q(0).start(); cp_q(1).start(); cp_win.start()
    cp_k(0).start(); cp_v(0).start(); cp_sk(0).start()

    sh = sh_ref[...].astype(f32)
    dvec = d_ref[...].astype(f32).reshape(1, D)
    bcol_s[...] = jnp.broadcast_to(b_ref[...].astype(f32).reshape(1, S), (128, S)).T
    k_s[0:8, :] = jnp.zeros((8, D), U32)

    def run(steps, pieces):
        for s_, step in enumerate(steps):
            acc = step()
            never = acc[0:8, 0:128] > jnp.inf
            lo, hi = s_ * len(pieces) // len(steps), (s_ + 1) * len(pieces) // len(steps)
            for piece in pieces[lo:hi]:
                piece(lambda c: jnp.where(jnp.broadcast_to(never[0:1], c.shape) if hasattr(c, 'shape') and c.shape != (8, 128) else never, 0.0 if not hasattr(c, 'dtype') else jnp.zeros_like(c), c))

    def lanes(c):
        return slice(c * 128, (c + 1) * 128)

    def xn_piece(j, g, gc=None):
        hr = pl.ds(pl.multiple_of(j * (RB // 2) + g * 8, 8), 8)
        x = q_s[hr, :]
        if gc is not None:
            x = jnp.concatenate([x[:, lanes(c)] for c in range(D // 128)], 1)
        x = _unp(x).astype(f32)
        xn_s[hr, :] = _pk(_ln(x))

    cp_q(0).wait()
    for g in range(RB // 16):
        xn_piece(0, g)
    cp_win.wait()
    cp_k(1).start(); cp_v(1).start(); cp_sk(1).start(); cp_q(2).start()

    def loop_a(i, carry):
        r, hr = rows(i), hrows(i)
        @pl.when(i + 2 < NB)
        def _():
            cp_k(i + 2).start(); cp_v(i + 2).start(); cp_sk(i + 2).start()
        @pl.when(i + 3 < NB)
        def _():
            cp_q(i + 3).start()
        @pl.when(i + 3 >= NB)
        def _():
            cp_wsp(i + 3 - NB).start()
        @pl.when(i + 1 < NB)
        def _():
            cp_q(i + 1).wait()
        cp_k(i).wait(); cp_v(i).wait(); cp_sk(i).wait()
        nxt = jnp.minimum(i + 1, NB - 1)

        def step(n, m):
            def f():
                hm = pl.ds(pl.multiple_of(i * (RB // 2) + m * (MA // 2), 8), MA // 2)
                d = jnp.dot(_unp(xn_s[hm, :]), _unp(win_s[:, lanes(n)]), preferred_element_type=f32)
                z = _gelu(d)
                if n < FH // 128:
                    z1_s[hm, lanes(n)] = _pk(z)
                else:
                    z2f_s[m * MA:(m + 1) * MA, lanes(n - FH // 128)] = z
                return d
            return f

        def ln_piece(g):
            def f(gc):
                z = jnp.concatenate([z2f_s[g * 16:(g + 1) * 16, lanes(c)] for c in range(FH // 128)], 1)
                z2_s[pl.ds(pl.multiple_of(i * (RB // 2) + g * 8, 8), 8), :] = _pk(_ln(z))
            return f

        def kv_piece(c, g):
            def f(gc):
                h0 = pl.multiple_of(i * (RB // 2) + g * (KV // 2), 8)
                kk = _unp(gc(k_s[pl.ds(h0, KV // 2 + 8), lanes(c)])).astype(f32)[8:]
                w = [sh[t:t + 1, lanes(c)] for t in range(4)]
                acc = kk[8:] * w[0]
                for t in range(1, 4):
                    acc = acc + pltpu.roll(kk, t, 0)[8:] * w[t]
                kv_s[pl.ds(pl.multiple_of(i * RB + g * KV, 8), KV), lanes(c)] = acc * _unp(v_s[pl.ds(h0, KV // 2), lanes(c)]).astype(f32)
            return f

        def kt_piece(c, g):
            def f(gc):
                t0 = pl.ds(pl.multiple_of(i * RB + g * 128, 128), 128)
                kt_s[t0, lanes(c)] = _unp(ssmk_s[c * 64:(c + 1) * 64, t0]).astype(f32).T
            return f

        nt = FH // 128
        early = [kv_piece(c, g) for c in range(D // 128) for g in range(RB // KV)]
        early += [kt_piece(c, g) for c in range(D // 128) for g in range(RB // 128)]
        late = [ln_piece(g) for g in range(RB // 16)]
        late += [functools.partial(xn_piece, nxt, g) for g in range(RB // 16)]
        run([step(n, m) for n in range(nt, 2 * nt) for m in range(RB // MA)], early)
        run([step(n, m) for n in range(nt) for m in range(RB // MA)], late)
        return carry
    jax.lax.fori_loop(0, NB, loop_a, 0)

    def spatial_steps(i, tiles, MS, KC):
        steps = []
        for n in tiles:
            for m in range(RB // MS):
                box = [None]
                r = pl.ds(pl.multiple_of(i * RB + m * MS, MS), MS)
                hr = pl.ds(pl.multiple_of(i * (RB // 2) + m * (MS // 2), MS // 2), MS // 2)
                for k in range(S // KC):
                    def f(n=n, k=k, box=box, r=r, hr=hr):
                        d = jnp.dot(_unp(wsp_s[hr, k * KC:(k + 1) * KC]), _unp(z2_s[k * KC // 2:(k + 1) * KC // 2, lanes(n)]),
                                    preferred_element_type=f32)
                        box[0] = d if k == 0 else box[0] + d
                        if k == S // KC - 1:
                            h_s[hr, lanes(n)] = _pk(_unp(z1_s[hr, lanes(n)]).astype(f32) * (box[0] + bcol_s[r, :]))
                        return box[0]
                    steps.append(f)
        return steps

    cp_g.start(); cp_gi.start()

    def loop_b(i, carry):
        @pl.when(i + 3 < NB)
        def _():
            cp_wsp(i + 3).start()
        @pl.when(i + 3 == NB)
        def _():
            cp_wout.start()
        cp_wsp(i).wait()
        r0 = pl.multiple_of(i * 8, 8)
        pieces = []
        for u, (src, dst) in enumerate(((kv_s, ax_s), (kt_s, ak_s)) * (D // 128)):
            c = u // 2
            def p1(p, u=u, c=c, src=src):
                def f(gc):
                    Q = _dft8([src[pl.ds((4 * m + p) * N2 + r0, 8), lanes(c)] for m in range(8)], gc)
                    for q in range(8):
                        t_s[u % 10, p * 8 + q, 0:8, :] = Q[q][0]
                        t_s[u % 10, p * 8 + q, 8:16, :] = Q[q][1]
                return f
            def p2(q, u=u, c=c, dst=dst):
                def f(gc):
                    o = _radix4([(t_s[u % 10, p * 8 + q, 0:8, :], t_s[u % 10, p * 8 + q, 8:16, :]) for p in range(4)], q, gc)
                    for j in range(4):
                        dst[q + 8 * j, pl.ds(r0, 8), lanes(c)] = _pk(jnp.concatenate(o[j], 0))
                return f
            pieces += [p1(p) for p in range(4)] + [p2(q) for q in range(8)]
        run(spatial_steps(i, (0, 1, 2), 64, 256), pieces)
        return carry
    jax.lax.fori_loop(0, NB, loop_b, 0)

    cp_g.wait(); cp_gi.wait()

    def loop_c(i, carry):
        sp = spatial_steps(i, (3,), 256, 256)
        for u in range(4):
            f = i * 4 + u
            gf = _unp(g_s[f])
            X = jnp.dot(gf, _unp(ax_s[f]), preferred_element_type=f32)
            K = jnp.dot(gf, _unp(ak_s[f]), preferred_element_type=f32)
            for st in sp[u * len(sp) // 4:(u + 1) * len(sp) // 4]:
                st()
            xr, xi, kr, ki = X[:N2], X[N2:], K[:N2], K[N2:]
            Y = jnp.concatenate([xr * kr - xi * ki, xr * ki + xi * kr], 0).astype(bf16)
            b_s[f] = jnp.dot(_unp(gi_s[f]), Y, preferred_element_type=f32)
        return carry
    jax.lax.fori_loop(0, NB, loop_c, 0)

    def loop_d(i, carry):
        rb = pl.multiple_of(i * 16, 16)
        pieces = []
        for c in range(D // 128):
            def p1(q, c=c):
                def f(gc):
                    z = gc(0.0)
                    o = _radix4_t([(b_s[q + 8 * j, pl.ds(rb, 8), lanes(c)] + z, b_s[q + 8 * j, pl.ds(rb + 8, 8), lanes(c)] + z)
                                   for j in range(4)], q)
                    for p in range(4):
                        t_s[c % 3, p * 8 + q, 0:8, :] = o[p][0]
                        t_s[c % 3, p * 8 + q, 8:16, :] = o[p][1]
                return f
            def p2(p, c=c):
                def f(gc):
                    z = gc(0.0)
                    y = _dft8_t([(t_s[c % 3, p * 8 + q, 0:8, :] + z, t_s[c % 3, p * 8 + q, 8:16, :] + z) for q in range(8)])
                    for m in range(8):
                        y_s[pl.ds(pl.multiple_of((4 * m + p) * N2 + i * 8, 8), 8), lanes(c)] = y[m]
                return f
            pieces += [p1(q) for q in range(8)] + [p2(p) for p in range(4)]
        run(spatial_steps(i, (4, 5), 256, 128), pieces)
        return carry
    jax.lax.fori_loop(0, NB, loop_d, 0)

    cp_wout.wait()

    def loop_e(i, carry):
        r, hr = rows(i), hrows(i)
        o = jnp.dot(_unp(h_s[hr, :]), _unp(wout_s[...]), preferred_element_type=f32)
        ho = 0.5 * o
        gate = ho * jnp.tanh(ho) + ho
        y = y_s[r, :] + kv_s[r, :] * dvec
        o_s[hr, :] = _pk(_unp(q_s[hr, :]).astype(f32) + _unp(xn_s[hr, :]).astype(f32) * y * gate)
        cp_o(i).start()
        return carry
    jax.lax.fori_loop(0, NB, loop_e, 0)
    for i in range(NB):
        cp_o(i).wait()


@jax.jit
def pallas_recurrent_scan__ssm_conv_h3__mixer_gmlp__prompt_kernel(
    A_q: jax.Array,
    A_k: jax.Array,
    A_v: jax.Array,
    A_shift_k: jax.Array,
    A_ssm_k: jax.Array,
    A_ssm_D: jax.Array,
    B_x: jax.Array,
    B_w_in: jax.Array,
    B_w_sp: jax.Array,
    B_b_sp: jax.Array,
    B_w_out: jax.Array,
):
    del B_x
    f32 = jnp.float32
    hbm = pl.BlockSpec(memory_space=pl.ANY)
    vm = pl.BlockSpec(memory_space=pltpu.VMEM)
    out = pl.pallas_call(
        _kernel,
        out_shape=jax.ShapeDtypeStruct((S, D), A_q.dtype),
        in_specs=[hbm, hbm, hbm, vm, hbm, vm, hbm, hbm, vm, hbm, hbm, hbm],
        out_specs=hbm,
        scratch_shapes=[
            pltpu.VMEM((S // 2, D), U32),
            pltpu.VMEM((S // 2 + 8, D), U32),
            pltpu.VMEM((S // 2, D), U32),
            pltpu.VMEM((D // 2, S), U32),
            pltpu.VMEM((D // 2, F), U32),
            pltpu.VMEM((S // 2, S), U32),
            pltpu.VMEM((FH // 2, D), U32),
            pltpu.VMEM((N1, N2, 2 * N2), U32),
            pltpu.VMEM((N1, N2, 2 * N2), U32),
            pltpu.VMEM((S // 2, D), U32),
            pltpu.VMEM((S // 2, D), U32),
            pltpu.VMEM((S // 2, FH), U32),
            pltpu.VMEM((S // 2, FH), U32),
            pltpu.VMEM((S // 2, FH), U32),
            pltpu.VMEM((S, D), f32),
            pltpu.VMEM((S, D), f32),
            pltpu.VMEM((N1, N2, D), U32),
            pltpu.VMEM((N1, N2, D), U32),
            pltpu.VMEM((N1, 2 * N2, D), f32),
            pltpu.VMEM((S, D), f32),
            pltpu.VMEM((S, 128), f32),
            pltpu.VMEM((RB, FH), f32),
            pltpu.VMEM((10, N1, 16, 128), f32),
            pltpu.SemaphoreType.DMA((NB,)),
            pltpu.SemaphoreType.DMA((NB,)),
            pltpu.SemaphoreType.DMA((NB,)),
            pltpu.SemaphoreType.DMA((NB,)),
            pltpu.SemaphoreType.DMA((S // SB,)),
            pltpu.SemaphoreType.DMA((NB,)),
            pltpu.SemaphoreType.DMA((4,)),
        ],
        compiler_params=pltpu.CompilerParams(vmem_limit_bytes=120 << 20),
    )(A_q.reshape(S, D), A_k.reshape(S, D), A_v.reshape(S, D), A_shift_k.T, A_ssm_k,
      A_ssm_D, B_w_in, B_w_sp, B_b_sp, B_w_out, _G_FWD, _G_INV)
    return out.reshape(A_q.shape)
```

```python
import functools
import numpy as np
import jax
import jax.numpy as jnp
import jax.experimental.pallas as pl
import jax.experimental.pallas.tpu as pltpu

S, D, F, FH = 2048, 640, 1536, 768
N1, N2 = 32, 64
EPS = 1e-5


def _cs(num, den):
    a = 2 * np.pi * num / den
    return float(np.cos(a)), float(np.sin(a))


_C1, _S1 = _cs(1, 16)
_C2 = float(np.sqrt(0.5))
_C3, _S3 = _cs(3, 16)


def _rot(a, b, c, s):
    return a * c - b * s, a * s + b * c


def _rot_t(a, b, c, s):
    return a * c + b * s, b * c - a * s


def _dft4(xs, C):
    c1, s1, c2, c3, s3 = C
    x0, x1, x2, x3 = xs
    y1r, y1i = x1 * c1, x1 * s1
    t2 = x2 * c2
    y3r, y3i = x3 * c3, x3 * s3
    ar, br = x0 + t2, x0 - t2
    cr, ci = y1r + y3r, y1i + y3i
    dr, di = y1r - y3r, y1i - y3i
    return [(ar + cr, t2 + ci), (br + di, -(t2 + dr)), (ar - cr, t2 - ci), (br - di, dr - t2)]


def _dft8(xs, gc):
    C = [gc(c) for c in (_C1, _S1, _C2, _C3, _S3)]
    E, O = _dft4(xs[0::2], C), _dft4(xs[1::2], C)
    out = [None] * 8
    for f in range(4):
        tr, ti = _rot(*O[f], *_cs(-(4 * f - 1), 32))
        out[f] = (E[f][0] + tr, E[f][1] + ti)
        out[f + 4] = (E[f][0] - tr, E[f][1] - ti)
    return out


def _radix4(Q, f, gc):
    y = [Q[0]]
    for p in range(1, 4):
        c, s = _cs(-p * (4 * f - 1), 4 * N1)
        y.append(_rot(*Q[p], gc(c), gc(s)))
    ar, ai = y[0][0] + y[2][0], y[0][1] + y[2][1]
    br, bi = y[0][0] - y[2][0], y[0][1] - y[2][1]
    cr, ci = y[1][0] + y[3][0], y[1][1] + y[3][1]
    dr, di = y[1][0] - y[3][0], y[1][1] - y[3][1]
    return [(ar + cr, ai + ci), (br + di, bi - dr), (ar - cr, ai - ci), (br - di, bi + dr)]


def _radix4_t(o, f):
    o0, o1, o2, o3 = o
    ar, ai = o0[0] + o2[0], o0[1] + o2[1]
    cr, ci = o0[0] - o2[0], o0[1] - o2[1]
    br, bi = o1[0] + o3[0], o1[1] + o3[1]
    di, dr = o1[0] - o3[0], o3[1] - o1[1]
    y = [(ar + br, ai + bi), (cr + dr, ci + di), (ar - br, ai - bi), (cr - dr, ci - di)]
    return [y[0]] + [_rot_t(*y[p], *_cs(-p * (4 * f - 1), 4 * N1)) for p in range(1, 4)]


def _dft4_t(B):
    (a0r, a0i), (a1r, a1i), (a2r, a2i), (a3r, a3i) = B
    ar, cr = a0r + a2r, a0r - a2r
    ai, ci = a0i + a2i, a0i - a2i
    br, di = a1r + a3r, a1r - a3r
    dr, m = a3i - a1i, a1i + a3i
    return [ar + br, (cr + dr) * _C1 + (ci + di) * _S1, ((ar - br) + (ai - m)) * _C2, (cr - dr) * _C3 + (ci - di) * _S3]


def _dft8_t(B):
    E, O = [None] * 4, [None] * 4
    for f in range(4):
        E[f] = (B[f][0] + B[f + 4][0], B[f][1] + B[f + 4][1])
        O[f] = _rot_t(B[f][0] - B[f + 4][0], B[f][1] - B[f + 4][1], *_cs(-(4 * f - 1), 32))
    out = [None] * 8
    out[0::2] = _dft4_t(E)
    out[1::2] = _dft4_t(O)
    return out


def _stage2_tables():
    f1 = np.arange(N1)[:, None, None]
    f2 = np.arange(N2)[None, :, None]
    n2 = np.arange(N2)[None, None, :]
    ph = -2 * np.pi * (n2 * (f1 - 0.25) / S + n2 * f2 / N2)
    gr, gi = np.cos(ph), np.sin(ph)
    g = np.concatenate([np.concatenate([gr, -gi], 2), np.concatenate([gi, gr], 2)], 1)
    perm = np.arange(2 * N2).reshape(2, N2 // 8, 8).transpose(1, 0, 2).reshape(-1)
    g = g[:, :, perm]
    ginv = np.transpose(g, (0, 2, 1)) / S
    return g.astype(jnp.bfloat16), np.ascontiguousarray(ginv).astype(jnp.bfloat16)


_G_FWD, _G_INV = _stage2_tables()


def _ln(x):
    m = jnp.mean(x, axis=-1, keepdims=True)
    xc = x - m
    v = jnp.mean(xc * xc, axis=-1, keepdims=True)
    return xc * jax.lax.rsqrt(v + EPS)


def _gelu(x):
    c = float(np.sqrt(2.0 / np.pi))
    u = x * (c + (c * 0.044715) * (x * x))
    return (0.5 * x) * (1.0 + jnp.tanh(u))


RB = 256
NB = S // RB
SB = RB
MA = 256
KV = 16
MS = 128
KC = 256
U32 = jnp.uint32


def _unp(x):
    return pltpu.bitcast(x, jnp.bfloat16)


def _pk(x):
    return pltpu.bitcast(x.astype(jnp.bfloat16), U32)


def _kernel(q_hbm, k_hbm, v_hbm, sh_ref, ssmk_hbm, d_ref, win_hbm, wsp_hbm, b_ref, wout_hbm,
            g_hbm, gi_hbm, o_hbm,
            q_s, k_s, v_s, ssmk_s, win_s, wsp_s, wout_s, g_s, gi_s, o_s,
            xn_s, z1_s, z2_s, h_s, kv_s, kt_s, ax_s, ak_s, b_s, y_s, bcol_s, z2f_s, t_s,
            sem_q, sem_k, sem_v, sem_sk, sem_wsp, sem_o, sem_m):
    f32, bf16 = jnp.float32, jnp.bfloat16
    q_hbm, k_hbm, v_hbm, ssmk_hbm, win_hbm, wsp_hbm, wout_hbm, g_hbm, gi_hbm, o_hbm = (
        r.bitcast(U32) for r in
        (q_hbm, k_hbm, v_hbm, ssmk_hbm, win_hbm, wsp_hbm, wout_hbm, g_hbm, gi_hbm, o_hbm))

    def rows(i, n=RB):
        return pl.ds(pl.multiple_of(i * n, n), n)

    def hrows(i, n=RB):
        return rows(i, n // 2)

    def cp_q(i): return pltpu.make_async_copy(q_hbm.at[hrows(i)], q_s.at[hrows(i)], sem_q.at[i])
    def cp_k(i): return pltpu.make_async_copy(k_hbm.at[hrows(i)], k_s.at[pl.ds(pl.multiple_of(8 + i * (RB // 2), 8), RB // 2)], sem_k.at[i])
    def cp_v(i): return pltpu.make_async_copy(v_hbm.at[hrows(i)], v_s.at[hrows(i)], sem_v.at[i])
    def cp_sk(i): return pltpu.make_async_copy(ssmk_hbm.at[:, rows(i)], ssmk_s.at[:, rows(i)], sem_sk.at[i])
    def cp_wsp(i): return pltpu.make_async_copy(wsp_hbm.at[hrows(i, SB)], wsp_s.at[hrows(i, SB)], sem_wsp.at[i])
    def cp_o(i): return pltpu.make_async_copy(o_s.at[hrows(i)], o_hbm.at[hrows(i)], sem_o.at[i])
    cp_win = pltpu.make_async_copy(win_hbm, win_s, sem_m.at[0])
    cp_wout = pltpu.make_async_copy(wout_hbm, wout_s, sem_m.at[1])
    cp_g = pltpu.make_async_copy(g_hbm, g_s, sem_m.at[2])
    cp_gi = pltpu.make_async_copy(gi_hbm, gi_s, sem_m.at[3])

    cp_q(0).start(); cp_q(1).start(); cp_win.start()
    cp_k(0).start(); cp_v(0).start(); cp_sk(0).start()

    sh = sh_ref[...].astype(f32)
    dvec = d_ref[...].astype(f32).reshape(1, D)
    bcol_s[...] = jnp.broadcast_to(b_ref[...].astype(f32).reshape(1, S), (128, S)).T
    k_s[0:8, :] = jnp.zeros((8, D), U32)

    def run(steps, pieces):
        for s_, step in enumerate(steps):
            acc = step()
            never = acc[0:8, 0:128] > jnp.inf
            lo, hi = s_ * len(pieces) // len(steps), (s_ + 1) * len(pieces) // len(steps)
            for piece in pieces[lo:hi]:
                piece(lambda c: jnp.where(jnp.broadcast_to(never[0:1], c.shape) if hasattr(c, 'shape') and c.shape != (8, 128) else never, 0.0 if not hasattr(c, 'dtype') else jnp.zeros_like(c), c))

    def lanes(c):
        return slice(c * 128, (c + 1) * 128)

    def xn_piece(j, g, gc=None):
        hr = pl.ds(pl.multiple_of(j * (RB // 2) + g * 8, 8), 8)
        x = q_s[hr, :]
        if gc is not None:
            x = jnp.concatenate([x[:, lanes(c)] for c in range(D // 128)], 1)
        x = _unp(x).astype(f32)
        xn_s[hr, :] = _pk(_ln(x))

    cp_q(0).wait()
    for g in range(RB // 16):
        xn_piece(0, g)
    cp_win.wait()
    cp_k(1).start(); cp_v(1).start(); cp_sk(1).start(); cp_q(2).start()

    def loop_a(i, carry):
        r, hr = rows(i), hrows(i)
        @pl.when(i + 2 < NB)
        def _():
            cp_k(i + 2).start(); cp_v(i + 2).start(); cp_sk(i + 2).start()
        @pl.when(i + 3 < NB)
        def _():
            cp_q(i + 3).start()
        @pl.when(i + 3 >= NB)
        def _():
            cp_wsp(i + 3 - NB).start()
        @pl.when(i + 1 < NB)
        def _():
            cp_q(i + 1).wait()
        cp_k(i).wait(); cp_v(i).wait(); cp_sk(i).wait()
        nxt = jnp.minimum(i + 1, NB - 1)

        def step(n, m):
            def f():
                hm = pl.ds(pl.multiple_of(i * (RB // 2) + m * (MA // 2), 8), MA // 2)
                d = jnp.dot(_unp(xn_s[hm, :]), _unp(win_s[:, lanes(n)]), preferred_element_type=f32)
                z = _gelu(d)
                if n < FH // 128:
                    z1_s[hm, lanes(n)] = _pk(z)
                else:
                    z2f_s[m * MA:(m + 1) * MA, lanes(n - FH // 128)] = z
                return d
            return f

        def ln_piece(g):
            def f(gc):
                z = jnp.concatenate([z2f_s[g * 16:(g + 1) * 16, lanes(c)] for c in range(FH // 128)], 1)
                z2_s[pl.ds(pl.multiple_of(i * (RB // 2) + g * 8, 8), 8), :] = _pk(_ln(z))
            return f

        def kv_piece(c, g):
            def f(gc):
                h0 = pl.multiple_of(i * (RB // 2) + g * (KV // 2), 8)
                kk = _unp(gc(k_s[pl.ds(h0, KV // 2 + 8), lanes(c)])).astype(f32)[8:]
                w = [sh[t:t + 1, lanes(c)] for t in range(4)]
                acc = kk[8:] * w[0]
                for t in range(1, 4):
                    acc = acc + pltpu.roll(kk, t, 0)[8:] * w[t]
                kv_s[pl.ds(pl.multiple_of(i * RB + g * KV, 8), KV), lanes(c)] = acc * _unp(v_s[pl.ds(h0, KV // 2), lanes(c)]).astype(f32)
            return f

        def kt_piece(c, g):
            def f(gc):
                t0 = pl.ds(pl.multiple_of(i * RB + g * 128, 128), 128)
                kt_s[t0, lanes(c)] = _unp(ssmk_s[c * 64:(c + 1) * 64, t0]).astype(f32).T
            return f

        nt = FH // 128
        early = [kv_piece(c, g) for c in range(D // 128) for g in range(RB // KV)]
        early += [kt_piece(c, g) for c in range(D // 128) for g in range(RB // 128)]
        late = [ln_piece(g) for g in range(RB // 16)]
        late += [functools.partial(xn_piece, nxt, g) for g in range(RB // 16)]
        run([step(n, m) for n in range(nt, 2 * nt) for m in range(RB // MA)], early)
        run([step(n, m) for n in range(nt) for m in range(RB // MA)], late)
        return carry
    jax.lax.fori_loop(0, NB, loop_a, 0)

    def spatial_steps(i, tiles, MS, KC):
        steps = []
        for n in tiles:
            for m in range(RB // MS):
                box = [None]
                r = pl.ds(pl.multiple_of(i * RB + m * MS, MS), MS)
                hr = pl.ds(pl.multiple_of(i * (RB // 2) + m * (MS // 2), MS // 2), MS // 2)
                for k in range(S // KC):
                    def f(n=n, k=k, box=box, r=r, hr=hr):
                        d = jnp.dot(_unp(wsp_s[hr, k * KC:(k + 1) * KC]), _unp(z2_s[k * KC // 2:(k + 1) * KC // 2, lanes(n)]),
                                    preferred_element_type=f32)
                        box[0] = d if k == 0 else box[0] + d
                        if k == S // KC - 1:
                            h_s[hr, lanes(n)] = _pk(_unp(z1_s[hr, lanes(n)]).astype(f32) * (box[0] + bcol_s[r, :]))
                        return box[0]
                    steps.append(f)
        return steps

    cp_g.start(); cp_gi.start()

    def loop_b(i, carry):
        @pl.when(i + 3 < NB)
        def _():
            cp_wsp(i + 3).start()
        @pl.when(i + 3 == NB)
        def _():
            cp_wout.start()
        cp_wsp(i).wait()
        r0 = pl.multiple_of(i * 8, 8)
        pieces = []
        for u, (src, dst) in enumerate(((kv_s, ax_s), (kt_s, ak_s)) * (D // 128)):
            c = u // 2
            def p1(p, u=u, c=c, src=src):
                def f(gc):
                    Q = _dft8([src[pl.ds((4 * m + p) * N2 + r0, 8), lanes(c)] for m in range(8)], gc)
                    for q in range(8):
                        t_s[u % 10, p * 8 + q, 0:8, :] = Q[q][0]
                        t_s[u % 10, p * 8 + q, 8:16, :] = Q[q][1]
                return f
            def p2(q, u=u, c=c, dst=dst):
                def f(gc):
                    o = _radix4([(t_s[u % 10, p * 8 + q, 0:8, :], t_s[u % 10, p * 8 + q, 8:16, :]) for p in range(4)], q, gc)
                    for j in range(4):
                        dst[q + 8 * j, pl.ds(r0, 8), lanes(c)] = _pk(jnp.concatenate(o[j], 0))
                return f
            pieces += [p1(p) for p in range(4)] + [p2(q) for q in range(8)]
        run(spatial_steps(i, (0, 1, 2), 64, 256), pieces)
        return carry
    jax.lax.fori_loop(0, NB, loop_b, 0)

    cp_g.wait(); cp_gi.wait()

    def loop_c(i, carry):
        sp = spatial_steps(i, (3,), 256, 256)
        for u in range(4):
            f = i * 4 + u
            gf = _unp(g_s[f])
            X = jnp.dot(gf, _unp(ax_s[f]), preferred_element_type=f32)
            K = jnp.dot(gf, _unp(ak_s[f]), preferred_element_type=f32)
            for st in sp[u * len(sp) // 4:(u + 1) * len(sp) // 4]:
                st()
            xr, xi, kr, ki = X[:N2], X[N2:], K[:N2], K[N2:]
            Y = jnp.concatenate([xr * kr - xi * ki, xr * ki + xi * kr], 0).astype(bf16)
            b_s[f] = jnp.dot(_unp(gi_s[f]), Y, preferred_element_type=f32)
        return carry
    jax.lax.fori_loop(0, NB, loop_c, 0, unroll=2)

    def loop_d(i, carry):
        rb = pl.multiple_of(i * 16, 16)
        pieces = []
        for c in range(D // 128):
            def p1(q, c=c):
                def f(gc):
                    z = gc(0.0)
                    o = _radix4_t([(b_s[q + 8 * j, pl.ds(rb, 8), lanes(c)] + z, b_s[q + 8 * j, pl.ds(rb + 8, 8), lanes(c)] + z)
                                   for j in range(4)], q)
                    for p in range(4):
                        t_s[c % 3, p * 8 + q, 0:8, :] = o[p][0]
                        t_s[c % 3, p * 8 + q, 8:16, :] = o[p][1]
                return f
            def p2(p, c=c):
                def f(gc):
                    z = gc(0.0)
                    y = _dft8_t([(t_s[c % 3, p * 8 + q, 0:8, :] + z, t_s[c % 3, p * 8 + q, 8:16, :] + z) for q in range(8)])
                    for m in range(8):
                        y_s[pl.ds(pl.multiple_of((4 * m + p) * N2 + i * 8, 8), 8), lanes(c)] = y[m]
                return f
            pieces += [p1(q) for q in range(8)] + [p2(p) for p in range(4)]
        run(spatial_steps(i, (4, 5), 256, 128), pieces)
        return carry
    jax.lax.fori_loop(0, NB, loop_d, 0)

    cp_wout.wait()

    def loop_e(i, carry):
        r, hr = rows(i, 2 * RB), hrows(i, 2 * RB)
        o = jnp.dot(_unp(h_s[hr, :]), _unp(wout_s[...]), preferred_element_type=f32)
        ho = 0.5 * o
        gate = ho * jnp.tanh(ho) + ho
        y = y_s[r, :] + kv_s[r, :] * dvec
        o_s[hr, :] = _pk(_unp(q_s[hr, :]).astype(f32) + _unp(xn_s[hr, :]).astype(f32) * y * gate)
        cp_o(2 * i).start(); cp_o(2 * i + 1).start()
        return carry
    jax.lax.fori_loop(0, NB // 2, loop_e, 0)
    for i in range(NB):
        cp_o(i).wait()


@jax.jit
def pallas_recurrent_scan__ssm_conv_h3__mixer_gmlp__prompt_kernel(
    A_q: jax.Array,
    A_k: jax.Array,
    A_v: jax.Array,
    A_shift_k: jax.Array,
    A_ssm_k: jax.Array,
    A_ssm_D: jax.Array,
    B_x: jax.Array,
    B_w_in: jax.Array,
    B_w_sp: jax.Array,
    B_b_sp: jax.Array,
    B_w_out: jax.Array,
):
    del B_x
    f32 = jnp.float32
    hbm = pl.BlockSpec(memory_space=pl.ANY)
    vm = pl.BlockSpec(memory_space=pltpu.VMEM)
    out = pl.pallas_call(
        _kernel,
        out_shape=jax.ShapeDtypeStruct((S, D), A_q.dtype),
        in_specs=[hbm, hbm, hbm, vm, hbm, vm, hbm, hbm, vm, hbm, hbm, hbm],
        out_specs=hbm,
        scratch_shapes=[
            pltpu.VMEM((S // 2, D), U32),
            pltpu.VMEM((S // 2 + 8, D), U32),
            pltpu.VMEM((S // 2, D), U32),
            pltpu.VMEM((D // 2, S), U32),
            pltpu.VMEM((D // 2, F), U32),
            pltpu.VMEM((S // 2, S), U32),
            pltpu.VMEM((FH // 2, D), U32),
            pltpu.VMEM((N1, N2, 2 * N2), U32),
            pltpu.VMEM((N1, N2, 2 * N2), U32),
            pltpu.VMEM((S // 2, D), U32),
            pltpu.VMEM((S // 2, D), U32),
            pltpu.VMEM((S // 2, FH), U32),
            pltpu.VMEM((S // 2, FH), U32),
            pltpu.VMEM((S // 2, FH), U32),
            pltpu.VMEM((S, D), f32),
            pltpu.VMEM((S, D), f32),
            pltpu.VMEM((N1, N2, D), U32),
            pltpu.VMEM((N1, N2, D), U32),
            pltpu.VMEM((N1, 2 * N2, D), f32),
            pltpu.VMEM((S, D), f32),
            pltpu.VMEM((S, 128), f32),
            pltpu.VMEM((RB, FH), f32),
            pltpu.VMEM((10, N1, 16, 128), f32),
            pltpu.SemaphoreType.DMA((NB,)),
            pltpu.SemaphoreType.DMA((NB,)),
            pltpu.SemaphoreType.DMA((NB,)),
            pltpu.SemaphoreType.DMA((NB,)),
            pltpu.SemaphoreType.DMA((S // SB,)),
            pltpu.SemaphoreType.DMA((NB,)),
            pltpu.SemaphoreType.DMA((4,)),
        ],
        compiler_params=pltpu.CompilerParams(vmem_limit_bytes=120 << 20),
    )(A_q.reshape(S, D), A_k.reshape(S, D), A_v.reshape(S, D), A_shift_k.T, A_ssm_k,
      A_ssm_D, B_w_in, B_w_sp, B_b_sp, B_w_out, _G_FWD, _G_INV)
    return out.reshape(A_q.shape)
```

```python
import functools
import numpy as np
import jax
import jax.numpy as jnp
import jax.experimental.pallas as pl
import jax.experimental.pallas.tpu as pltpu

S, D, F, FH = 2048, 640, 1536, 768
N1, N2 = 32, 64
EPS = 1e-5


def _cs(num, den):
    a = 2 * np.pi * num / den
    return float(np.cos(a)), float(np.sin(a))


_C1, _S1 = _cs(1, 16)
_C2 = float(np.sqrt(0.5))
_C3, _S3 = _cs(3, 16)


def _rot(a, b, c, s):
    return a * c - b * s, a * s + b * c


def _rot_t(a, b, c, s):
    return a * c + b * s, b * c - a * s


def _dft4(xs, C):
    c1, s1, c2, c3, s3 = C
    x0, x1, x2, x3 = xs
    y1r, y1i = x1 * c1, x1 * s1
    t2 = x2 * c2
    y3r, y3i = x3 * c3, x3 * s3
    ar, br = x0 + t2, x0 - t2
    cr, ci = y1r + y3r, y1i + y3i
    dr, di = y1r - y3r, y1i - y3i
    return [(ar + cr, t2 + ci), (br + di, -(t2 + dr)), (ar - cr, t2 - ci), (br - di, dr - t2)]


def _dft8(xs, gc):
    C = [gc(c) for c in (_C1, _S1, _C2, _C3, _S3)]
    E, O = _dft4(xs[0::2], C), _dft4(xs[1::2], C)
    out = [None] * 8
    for f in range(4):
        tr, ti = _rot(*O[f], *_cs(-(4 * f - 1), 32))
        out[f] = (E[f][0] + tr, E[f][1] + ti)
        out[f + 4] = (E[f][0] - tr, E[f][1] - ti)
    return out


def _radix4(Q, f, gc):
    y = [Q[0]]
    for p in range(1, 4):
        c, s = _cs(-p * (4 * f - 1), 4 * N1)
        y.append(_rot(*Q[p], gc(c), gc(s)))
    ar, ai = y[0][0] + y[2][0], y[0][1] + y[2][1]
    br, bi = y[0][0] - y[2][0], y[0][1] - y[2][1]
    cr, ci = y[1][0] + y[3][0], y[1][1] + y[3][1]
    dr, di = y[1][0] - y[3][0], y[1][1] - y[3][1]
    return [(ar + cr, ai + ci), (br + di, bi - dr), (ar - cr, ai - ci), (br - di, bi + dr)]


def _radix4_t(o, f):
    o0, o1, o2, o3 = o
    ar, ai = o0[0] + o2[0], o0[1] + o2[1]
    cr, ci = o0[0] - o2[0], o0[1] - o2[1]
    br, bi = o1[0] + o3[0], o1[1] + o3[1]
    di, dr = o1[0] - o3[0], o3[1] - o1[1]
    y = [(ar + br, ai + bi), (cr + dr, ci + di), (ar - br, ai - bi), (cr - dr, ci - di)]
    return [y[0]] + [_rot_t(*y[p], *_cs(-p * (4 * f - 1), 4 * N1)) for p in range(1, 4)]


def _dft4_t(B):
    (a0r, a0i), (a1r, a1i), (a2r, a2i), (a3r, a3i) = B
    ar, cr = a0r + a2r, a0r - a2r
    ai, ci = a0i + a2i, a0i - a2i
    br, di = a1r + a3r, a1r - a3r
    dr, m = a3i - a1i, a1i + a3i
    return [ar + br, (cr + dr) * _C1 + (ci + di) * _S1, ((ar - br) + (ai - m)) * _C2, (cr - dr) * _C3 + (ci - di) * _S3]


def _dft8_t(B):
    E, O = [None] * 4, [None] * 4
    for f in range(4):
        E[f] = (B[f][0] + B[f + 4][0], B[f][1] + B[f + 4][1])
        O[f] = _rot_t(B[f][0] - B[f + 4][0], B[f][1] - B[f + 4][1], *_cs(-(4 * f - 1), 32))
    out = [None] * 8
    out[0::2] = _dft4_t(E)
    out[1::2] = _dft4_t(O)
    return out


def _stage2_tables():
    f1 = np.arange(N1)[:, None, None]
    f2 = np.arange(N2)[None, :, None]
    n2 = np.arange(N2)[None, None, :]
    ph = -2 * np.pi * (n2 * (f1 - 0.25) / S + n2 * f2 / N2)
    gr, gi = np.cos(ph), np.sin(ph)
    g = np.concatenate([np.concatenate([gr, -gi], 2), np.concatenate([gi, gr], 2)], 1)
    perm = np.arange(2 * N2).reshape(2, N2 // 8, 8).transpose(1, 0, 2).reshape(-1)
    g = g[:, :, perm]
    ginv = np.transpose(g, (0, 2, 1)) / S
    return g.astype(jnp.bfloat16), np.ascontiguousarray(ginv).astype(jnp.bfloat16)


_G_FWD, _G_INV = _stage2_tables()


def _ln(x):
    m = jnp.mean(x, axis=-1, keepdims=True)
    xc = x - m
    v = jnp.mean(xc * xc, axis=-1, keepdims=True)
    return xc * jax.lax.rsqrt(v + EPS)


def _gelu(x):
    c = float(np.sqrt(2.0 / np.pi))
    u = x * (c + (c * 0.044715) * (x * x))
    return (0.5 * x) * (1.0 + jnp.tanh(u))


RB = 256
NB = S // RB
SB = RB
LAG = 1
MA = 256
KV = 16
MS = 128
KC = 256
U32 = jnp.uint32


def _unp(x):
    return pltpu.bitcast(x, jnp.bfloat16)


def _pk(x):
    return pltpu.bitcast(x.astype(jnp.bfloat16), U32)


def _kernel(q_hbm, k_hbm, v_hbm, sh_ref, ssmk_hbm, d_ref, win_hbm, wsp_hbm, b_ref, wout_hbm,
            g_hbm, gi_hbm, o_hbm,
            q_s, k_s, v_s, ssmk_s, win_s, wsp_s, wout_s, g_s, gi_s, o_s,
            xn_s, z1_s, z2_s, h_s, kv_s, kt_s, ax_s, ak_s, b_s, y_s, bcol_s, z2f_s, t_s,
            sem_q, sem_k, sem_v, sem_sk, sem_wsp, sem_o, sem_m):
    f32, bf16 = jnp.float32, jnp.bfloat16
    q_hbm, k_hbm, v_hbm, ssmk_hbm, win_hbm, wsp_hbm, wout_hbm, g_hbm, gi_hbm, o_hbm = (
        r.bitcast(U32) for r in
        (q_hbm, k_hbm, v_hbm, ssmk_hbm, win_hbm, wsp_hbm, wout_hbm, g_hbm, gi_hbm, o_hbm))

    def rows(i, n=RB):
        return pl.ds(pl.multiple_of(i * n, n), n)

    def hrows(i, n=RB):
        return rows(i, n // 2)

    def cp_q(i): return pltpu.make_async_copy(q_hbm.at[hrows(i)], q_s.at[hrows(i)], sem_q.at[i])
    def cp_k(i): return pltpu.make_async_copy(k_hbm.at[hrows(i)], k_s.at[pl.ds(pl.multiple_of(8 + i * (RB // 2), 8), RB // 2)], sem_k.at[i])
    def cp_v(i): return pltpu.make_async_copy(v_hbm.at[hrows(i)], v_s.at[hrows(i)], sem_v.at[i])
    def cp_sk(i): return pltpu.make_async_copy(ssmk_hbm.at[:, rows(i)], ssmk_s.at[:, rows(i)], sem_sk.at[i])
    def cp_wsp(i): return pltpu.make_async_copy(wsp_hbm.at[hrows(i, SB)], wsp_s.at[hrows(i, SB)], sem_wsp.at[i])
    def cp_o(i): return pltpu.make_async_copy(o_s.at[hrows(i)], o_hbm.at[hrows(i)], sem_o.at[i])
    cp_win = pltpu.make_async_copy(win_hbm, win_s, sem_m.at[0])
    cp_wout = pltpu.make_async_copy(wout_hbm, wout_s, sem_m.at[1])
    cp_g = pltpu.make_async_copy(g_hbm, g_s, sem_m.at[2])
    cp_gi = pltpu.make_async_copy(gi_hbm, gi_s, sem_m.at[3])

    cp_q(0).start(); cp_q(1).start(); cp_win.start()
    cp_k(0).start(); cp_v(0).start(); cp_sk(0).start()

    sh = sh_ref[...].astype(f32)
    dvec = d_ref[...].astype(f32).reshape(1, D)
    bcol_s[...] = jnp.broadcast_to(b_ref[...].astype(f32).reshape(1, S), (128, S)).T
    k_s[0:8, :] = jnp.zeros((8, D), U32)

    def run(steps, pieces, lag=LAG):
        nv = []
        for s_, step in enumerate(steps):
            acc = step()
            nv.append(acc[0:8, 0:128] > jnp.inf)
            never = nv[max(0, len(nv) - 1 - lag)]
            lo, hi = s_ * len(pieces) // len(steps), (s_ + 1) * len(pieces) // len(steps)
            for piece in pieces[lo:hi]:
                piece(lambda c: jnp.where(jnp.broadcast_to(never[0:1], c.shape) if hasattr(c, 'shape') and c.shape != (8, 128) else never, 0.0 if not hasattr(c, 'dtype') else jnp.zeros_like(c), c))

    def lanes(c):
        return slice(c * 128, (c + 1) * 128)

    def xn_piece(j, g, gc=None):
        hr = pl.ds(pl.multiple_of(j * (RB // 2) + g * 8, 8), 8)
        x = q_s[hr, :]
        if gc is not None:
            x = jnp.concatenate([x[:, lanes(c)] for c in range(D // 128)], 1)
        x = _unp(x).astype(f32)
        xn_s[hr, :] = _pk(_ln(x))

    cp_q(0).wait()
    for g in range(RB // 16):
        xn_piece(0, g)
    cp_win.wait()
    cp_k(1).start(); cp_v(1).start(); cp_sk(1).start(); cp_q(2).start()

    def loop_a(i, carry):
        r, hr = rows(i), hrows(i)
        @pl.when(i + 2 < NB)
        def _():
            cp_k(i + 2).start(); cp_v(i + 2).start(); cp_sk(i + 2).start()
        @pl.when(i + 3 < NB)
        def _():
            cp_q(i + 3).start()
        @pl.when(i + 3 >= NB)
        def _():
            cp_wsp(i + 3 - NB).start()
        @pl.when(i + 1 < NB)
        def _():
            cp_q(i + 1).wait()
        cp_k(i).wait(); cp_v(i).wait(); cp_sk(i).wait()
        nxt = jnp.minimum(i + 1, NB - 1)

        def step(n, m):
            def f():
                hm = pl.ds(pl.multiple_of(i * (RB // 2) + m * (MA // 2), 8), MA // 2)
                d = jnp.dot(_unp(xn_s[hm, :]), _unp(win_s[:, lanes(n)]), preferred_element_type=f32)
                z = _gelu(d)
                if n < FH // 128:
                    z1_s[hm, lanes(n)] = _pk(z)
                else:
                    z2f_s[m * MA:(m + 1) * MA, lanes(n - FH // 128)] = z
                return d
            return f

        def ln_piece(g):
            def f(gc):
                z = jnp.concatenate([z2f_s[g * 16:(g + 1) * 16, lanes(c)] for c in range(FH // 128)], 1)
                z2_s[pl.ds(pl.multiple_of(i * (RB // 2) + g * 8, 8), 8), :] = _pk(_ln(z))
            return f

        def kv_piece(c, g):
            def f(gc):
                h0 = pl.multiple_of(i * (RB // 2) + g * (KV // 2), 8)
                kk = _unp(gc(k_s[pl.ds(h0, KV // 2 + 8), lanes(c)])).astype(f32)[8:]
                w = [sh[t:t + 1, lanes(c)] for t in range(4)]
                acc = kk[8:] * w[0]
                for t in range(1, 4):
                    acc = acc + pltpu.roll(kk, t, 0)[8:] * w[t]
                kv_s[pl.ds(pl.multiple_of(i * RB + g * KV, 8), KV), lanes(c)] = acc * _unp(v_s[pl.ds(h0, KV // 2), lanes(c)]).astype(f32)
            return f

        def kt_piece(c, g):
            def f(gc):
                t0 = pl.ds(pl.multiple_of(i * RB + g * 128, 128), 128)
                kt_s[t0, lanes(c)] = _unp(ssmk_s[c * 64:(c + 1) * 64, t0]).astype(f32).T
            return f

        nt = FH // 128
        early = [kv_piece(c, g) for c in range(D // 128) for g in range(RB // KV)]
        early += [kt_piece(c, g) for c in range(D // 128) for g in range(RB // 128)]
        late = [ln_piece(g) for g in range(RB // 16)]
        late += [functools.partial(xn_piece, nxt, g) for g in range(RB // 16)]
        run([step(n, m) for n in range(nt, 2 * nt) for m in range(RB // MA)], early, 2)
        run([step(n, m) for n in range(nt) for m in range(RB // MA)], late, 2)
        return carry
    jax.lax.fori_loop(0, NB, loop_a, 0)

    def spatial_steps(i, tiles, MS, KC):
        steps = []
        for n in tiles:
            for m in range(RB // MS):
                box = [None]
                r = pl.ds(pl.multiple_of(i * RB + m * MS, MS), MS)
                hr = pl.ds(pl.multiple_of(i * (RB // 2) + m * (MS // 2), MS // 2), MS // 2)
                for k in range(S // KC):
                    def f(n=n, k=k, box=box, r=r, hr=hr):
                        d = jnp.dot(_unp(wsp_s[hr, k * KC:(k + 1) * KC]), _unp(z2_s[k * KC // 2:(k + 1) * KC // 2, lanes(n)]),
                                    preferred_element_type=f32)
                        box[0] = d if k == 0 else box[0] + d
                        if k == S // KC - 1:
                            h_s[hr, lanes(n)] = _pk(_unp(z1_s[hr, lanes(n)]).astype(f32) * (box[0] + bcol_s[r, :]))
                        return box[0]
                    steps.append(f)
        return steps

    cp_g.start(); cp_gi.start()

    def loop_b(i, carry):
        @pl.when(i + 3 < NB)
        def _():
            cp_wsp(i + 3).start()
        @pl.when(i + 3 == NB)
        def _():
            cp_wout.start()
        cp_wsp(i).wait()
        r0 = pl.multiple_of(i * 8, 8)
        pieces = []
        for u, (src, dst) in enumerate(((kv_s, ax_s), (kt_s, ak_s)) * (D // 128)):
            c = u // 2
            def p1(p, u=u, c=c, src=src):
                def f(gc):
                    Q = _dft8([src[pl.ds((4 * m + p) * N2 + r0, 8), lanes(c)] for m in range(8)], gc)
                    for q in range(8):
                        t_s[u % 10, p * 8 + q, 0:8, :] = Q[q][0]
                        t_s[u % 10, p * 8 + q, 8:16, :] = Q[q][1]
                return f
            def p2(q, u=u, c=c, dst=dst):
                def f(gc):
                    o = _radix4([(t_s[u % 10, p * 8 + q, 0:8, :], t_s[u % 10, p * 8 + q, 8:16, :]) for p in range(4)], q, gc)
                    for j in range(4):
                        dst[q + 8 * j, pl.ds(r0, 8), lanes(c)] = _pk(jnp.concatenate(o[j], 0))
                return f
            pieces += [p1(p) for p in range(4)] + [p2(q) for q in range(8)]
        run(spatial_steps(i, (0, 1, 2), 64, 256), pieces)
        return carry
    jax.lax.fori_loop(0, NB, loop_b, 0)

    cp_g.wait(); cp_gi.wait()

    def loop_c(i, carry):
        sp = spatial_steps(i, (3,), 256, 256)
        for u in range(4):
            f = i * 4 + u
            gf = _unp(g_s[f])
            X = jnp.dot(gf, _unp(ax_s[f]), preferred_element_type=f32)
            K = jnp.dot(gf, _unp(ak_s[f]), preferred_element_type=f32)
            for st in sp[u * len(sp) // 4:(u + 1) * len(sp) // 4]:
                st()
            xr, xi, kr, ki = X[:N2], X[N2:], K[:N2], K[N2:]
            Y = jnp.concatenate([xr * kr - xi * ki, xr * ki + xi * kr], 0).astype(bf16)
            b_s[f] = jnp.dot(_unp(gi_s[f]), Y, preferred_element_type=f32)
        return carry
    jax.lax.fori_loop(0, NB, loop_c, 0, unroll=2)

    def loop_d(i, carry):
        rb = pl.multiple_of(i * 16, 16)
        pieces = []
        for c in range(D // 128):
            def p1(q, c=c):
                def f(gc):
                    z = gc(0.0)
                    o = _radix4_t([(b_s[q + 8 * j, pl.ds(rb, 8), lanes(c)] + z, b_s[q + 8 * j, pl.ds(rb + 8, 8), lanes(c)] + z)
                                   for j in range(4)], q)
                    for p in range(4):
                        t_s[c % 3, p * 8 + q, 0:8, :] = o[p][0]
                        t_s[c % 3, p * 8 + q, 8:16, :] = o[p][1]
                return f
            def p2(p, c=c):
                def f(gc):
                    z = gc(0.0)
                    y = _dft8_t([(t_s[c % 3, p * 8 + q, 0:8, :] + z, t_s[c % 3, p * 8 + q, 8:16, :] + z) for q in range(8)])
                    for m in range(8):
                        y_s[pl.ds(pl.multiple_of((4 * m + p) * N2 + i * 8, 8), 8), lanes(c)] = y[m]
                return f
            pieces += [p1(q) for q in range(8)] + [p2(p) for p in range(4)]
        run(spatial_steps(i, (4, 5), 256, 128), pieces)
        return carry
    jax.lax.fori_loop(0, NB, loop_d, 0)

    cp_wout.wait()

    def loop_e(i, carry):
        r, hr = rows(i, 2 * RB), hrows(i, 2 * RB)
        o = jnp.dot(_unp(h_s[hr, :]), _unp(wout_s[...]), preferred_element_type=f32)
        ho = 0.5 * o
        gate = ho * jnp.tanh(ho) + ho
        y = y_s[r, :] + kv_s[r, :] * dvec
        o_s[hr, :] = _pk(_unp(q_s[hr, :]).astype(f32) + _unp(xn_s[hr, :]).astype(f32) * y * gate)
        cp_o(2 * i).start(); cp_o(2 * i + 1).start()
        return carry
    jax.lax.fori_loop(0, NB // 2, loop_e, 0)
    for i in range(NB):
        cp_o(i).wait()


@jax.jit
def pallas_recurrent_scan__ssm_conv_h3__mixer_gmlp__prompt_kernel(
    A_q: jax.Array,
    A_k: jax.Array,
    A_v: jax.Array,
    A_shift_k: jax.Array,
    A_ssm_k: jax.Array,
    A_ssm_D: jax.Array,
    B_x: jax.Array,
    B_w_in: jax.Array,
    B_w_sp: jax.Array,
    B_b_sp: jax.Array,
    B_w_out: jax.Array,
):
    del B_x
    f32 = jnp.float32
    hbm = pl.BlockSpec(memory_space=pl.ANY)
    vm = pl.BlockSpec(memory_space=pltpu.VMEM)
    out = pl.pallas_call(
        _kernel,
        out_shape=jax.ShapeDtypeStruct((S, D), A_q.dtype),
        in_specs=[hbm, hbm, hbm, vm, hbm, vm, hbm, hbm, vm, hbm, hbm, hbm],
        out_specs=hbm,
        scratch_shapes=[
            pltpu.VMEM((S // 2, D), U32),
            pltpu.VMEM((S // 2 + 8, D), U32),
            pltpu.VMEM((S // 2, D), U32),
            pltpu.VMEM((D // 2, S), U32),
            pltpu.VMEM((D // 2, F), U32),
            pltpu.VMEM((S // 2, S), U32),
            pltpu.VMEM((FH // 2, D), U32),
            pltpu.VMEM((N1, N2, 2 * N2), U32),
            pltpu.VMEM((N1, N2, 2 * N2), U32),
            pltpu.VMEM((S // 2, D), U32),
            pltpu.VMEM((S // 2, D), U32),
            pltpu.VMEM((S // 2, FH), U32),
            pltpu.VMEM((S // 2, FH), U32),
            pltpu.VMEM((S // 2, FH), U32),
            pltpu.VMEM((S, D), f32),
            pltpu.VMEM((S, D), f32),
            pltpu.VMEM((N1, N2, D), U32),
            pltpu.VMEM((N1, N2, D), U32),
            pltpu.VMEM((N1, 2 * N2, D), f32),
            pltpu.VMEM((S, D), f32),
            pltpu.VMEM((S, 128), f32),
            pltpu.VMEM((RB, FH), f32),
            pltpu.VMEM((10, N1, 16, 128), f32),
            pltpu.SemaphoreType.DMA((NB,)),
            pltpu.SemaphoreType.DMA((NB,)),
            pltpu.SemaphoreType.DMA((NB,)),
            pltpu.SemaphoreType.DMA((NB,)),
            pltpu.SemaphoreType.DMA((S // SB,)),
            pltpu.SemaphoreType.DMA((NB,)),
            pltpu.SemaphoreType.DMA((4,)),
        ],
        compiler_params=pltpu.CompilerParams(vmem_limit_bytes=120 << 20),
    )(A_q.reshape(S, D), A_k.reshape(S, D), A_v.reshape(S, D), A_shift_k.T, A_ssm_k,
      A_ssm_D, B_w_in, B_w_sp, B_b_sp, B_w_out, _G_FWD, _G_INV)
    return out.reshape(A_q.shape)
```
